```python
import jax
import jax.numpy as jnp

def _softmax(x, axis=-1):
    return jax.nn.softmax(x, axis=axis)

def _gelu(x):
    return jax.nn.gelu(x, approximate=True)

def _silu(x):
    return jax.nn.silu(x)

def _sigmoid(x):
    return jax.nn.sigmoid(x)

def _layernorm(x, axis=-1, eps=1e-05):
    m = jnp.mean(x, axis=axis, keepdims=True)
    v = jnp.var(x, axis=axis, keepdims=True)
    return (x - m) / jnp.sqrt(v + eps)

def _scatter_add(tgt, idx, src, axis=0):
    return tgt.at[idx].add(src)

def _segment_sum(src, seg, n):
    return jax.ops.segment_sum(src, seg, n)

class _Rng:

    def __init__(self, key):
        self._k = key

    def _next(self):
        self._k, sub = jax.random.split(self._k)
        return sub

    def normal(self, shape):
        return jax.random.normal(self._next(), shape, dtype=jnp.bfloat16)

    def randint(self, lo, hi, shape):
        return jax.random.randint(self._next(), shape, lo, hi, dtype=jnp.int32)

    def uniform(self, shape, lo=0.0, hi=1.0):
        return jax.random.uniform(self._next(), shape, jnp.bfloat16, lo, hi)

    def permutation(self, n):
        return jax.random.permutation(self._next(), n)
kernel_name = 'recurrent_scan__memory_aug_recurrent_mem_tr__moe_arch_mod__prompt'

def setup_inputs():
    _rng = _Rng(jax.random.key(int.from_bytes(__import__("os").urandom(4), "little")))
    _w = lambda a: (lambda t: t.astype(jnp.bfloat16) if jnp.issubdtype(t.dtype, jnp.floating) else t)(jnp.asarray(a))

    def _A_setup():
        B, S, Dm = (1, 2048, 640)
        H, Dh = (32, 128)
        M, seg = (8, 32)
        seg = min(seg, S)
        S = S // seg * seg
        return {'x': _w((lambda *s: _rng.normal(s) * 0.05)(B, S, Dm)), 'mem0': _w((lambda *s: _rng.normal(s) * 0.05)(B, M, Dm)), 'Wq': _w((lambda *s: _rng.normal(s) * 0.05)(Dm, H, Dh) * Dm ** (-0.5)), 'Wk': _w((lambda *s: _rng.normal(s) * 0.05)(Dm, H, Dh) * Dm ** (-0.5)), 'Wv': _w((lambda *s: _rng.normal(s) * 0.05)(Dm, H, Dh) * Dm ** (-0.5)), 'Wo': _w((lambda *s: _rng.normal(s) * 0.05)(H, Dh, Dm) * (H * Dh) ** (-0.5)), 'seg_len': seg}
    _A_in = _A_setup()

    def _B_setup():
        B, S, D, F, C = (1, 2048, 640, 1728, 8)
        return {'x': _w((lambda *s: _rng.normal(s) * 0.05)(B, S, D)), 'w_r': _w((lambda *s: _rng.normal(s) * 0.05)(D)), 'w_gate': _w((lambda *s: _rng.normal(s) * 0.05)(D, F)), 'w_up': _w((lambda *s: _rng.normal(s) * 0.05)(D, F)), 'w_down': _w((lambda *s: _rng.normal(s) * 0.05)(F, D))}
    _B_in = _B_setup()
    return {'A_x': _A_in['x'], 'A_mem0': _A_in['mem0'], 'A_Wq': _A_in['Wq'], 'A_Wk': _A_in['Wk'], 'A_Wv': _A_in['Wv'], 'A_Wo': _A_in['Wo'], 'A_seg_len': _A_in['seg_len'], 'B_x': _B_in['x'], 'B_w_r': _B_in['w_r'], 'B_w_gate': _B_in['w_gate'], 'B_w_up': _B_in['w_up'], 'B_w_down': _B_in['w_down']}

def reference(A_x, A_mem0, A_Wq, A_Wk, A_Wv, A_Wo, A_seg_len, B_x, B_w_r, B_w_gate, B_w_up, B_w_down):

    def _A_ref(x, mem0, Wq, Wk, Wv, Wo, seg_len):
        B, S, Dm = x.shape
        H, Dh = (Wq.shape[1], Wq.shape[2])
        M = mem0.shape[1]
        scale = Dh ** (-0.5)
        n_seg = S // seg_len
        L = M + seg_len
        idx = jnp.arange(L)
        mask = (idx[:, None] < M) | (idx[:, None] >= idx[None, :])
        mem = mem0
        outs = []
        for s in range(n_seg):
            xs = x[:, s * seg_len:(s + 1) * seg_len, :].copy()
            h = jnp.concatenate([mem, xs], axis=1)
            q = jnp.einsum('btd,dhe->bhte', h, Wq)
            k = jnp.einsum('btd,dhe->bhte', h, Wk)
            v = jnp.einsum('btd,dhe->bhte', h, Wv)
            scores = jnp.einsum('bhqe,bhke->bhqk', q, k) * scale
            scores = jnp.where(mask[None, None], scores, -1000000000.0)
            p = _softmax(scores, axis=-1)
            o = jnp.einsum('bhqk,bhke->bhqe', p, v)
            o = jnp.einsum('bhte,hed->btd', o, Wo)
            mem = o[:, :M, :].copy()
            outs.append(o[:, M:, :])
        return jnp.concatenate(outs, axis=1)

    def _B_ref(x, w_r, w_gate, w_up, w_down):
        B, S, D = x.shape
        C = 8
        r = x @ w_r
        idx = jnp.argsort(-r, axis=-1)[:, :C]
        idx_e = jnp.repeat(idx.reshape(B, C, 1), D, axis=2)
        x_sel = jnp.take_along_axis(x, idx_e, axis=1)
        g = _silu(x_sel @ w_gate)
        u = x_sel @ w_up
        y = g * u @ w_down
        r_sel = _sigmoid(jnp.take_along_axis(r, idx, axis=1))
        y = y * r_sel.reshape(B, C, 1)
        b_off = (jnp.arange(B) * S).reshape(B, 1)
        flat_idx = (idx + b_off).reshape(B * C)
        zero = (x * 0.0).reshape(B * S, D)
        upd = _scatter_add(zero, flat_idx, y.reshape(B * C, D), axis=0)
        return x + upd.reshape(B, S, D)
    x = A_x
    xn = _layernorm(x, axis=-1)
    s = _A_ref(xn, A_mem0, A_Wq, A_Wk, A_Wv, A_Wo, A_seg_len)
    g = _silu(_B_ref(xn, B_w_r, B_w_gate, B_w_up, B_w_down))
    return x + s * g
```

```python
import functools

import jax
import jax.numpy as jnp
import numpy as np
from jax import lax
from jax.experimental import pallas as pl
from jax.experimental.pallas import tpu as pltpu

_F32 = jnp.float32
_BF16 = jnp.bfloat16
_U32 = jnp.uint32
_NT = (((1,), (1,)), ((), ()))

_TOP_C = 8
_G = 4
_CH = 16
_LN_EPS = 1e-05


def _rnd(v):
    return v.astype(_BF16).astype(_F32)


def _silu(v):
    return v * jax.nn.sigmoid(v)


def _schedule(ng):
    toks = []
    for g in range(ng):
        toks.append(("A", g))
        if g >= 1:
            toks.append(("S", g - 1))
        if g >= 3:
            toks.append(("P", g - 3))
        toks.append(("W", g))
    tail = [[("S", ng - 1), ("P", ng - 3)], [("P", ng - 2)], [("P", ng - 1)]]
    o = 0
    for grp in tail:
        for _ in range(ng // 4):
            toks.append(("O", o))
            o += 1
        toks += grp
    while o < ng:
        toks.append(("O", o))
        o += 1
    return toks


def _kernel(x_hbm, mem0_ref, wq_hbm, wk_hbm, wv_hbm, wo_hbm, wr_ref, wg_hbm, wu_hbm, wd_hbm,
            out_hbm,
            xb, xn, gate, stg, w, wo, ring, wg, wu, wd, sbuf, obuf, sems, osem,
            *, seg, n_mem, heads, dh):
    S, D = xb.shape
    n_seg = S // seg
    L = seg + n_mem
    xrows = seg - n_mem
    pre = S - n_seg * xrows
    ring_rows = ring.shape[1]
    ring_off = ring_rows - pre
    n_chunk = 3 * heads // _CH
    n_col = D // 128
    ln_rows = (S - pre) // (n_chunk - 2)
    ng = heads // _G

    def x_copy(c):
        r0, n = (0, pre) if c == 0 else (pre + (c - 1) * ln_rows, ln_rows)
        return pltpu.make_async_copy(x_hbm.at[pl.ds(r0, n)], xb.at[pl.ds(r0, n)], sems.at[c])

    def x_copy_dyn(c):
        r0 = pl.multiple_of(pre + c * ln_rows, 16)
        return pltpu.make_async_copy(x_hbm.at[pl.ds(r0, ln_rows)], xb.at[pl.ds(r0, ln_rows)],
                                     sems.at[c + 1])

    sem_w = n_chunk - 1

    def w_copy(c):
        src = (wq_hbm, wk_hbm, wv_hbm)[c // (heads // _CH)].bitcast(_U32)
        h2 = (c % (heads // _CH)) * (_CH // 2)
        return pltpu.make_async_copy(src.at[:, pl.ds(h2, _CH // 2), :],
                                     stg.at[c].reshape(D, _CH // 2, dh), sems.at[sem_w + c])

    def w_wait_dyn(c):
        pltpu.make_async_copy(stg.at[c], stg.at[c], sems.at[sem_w + c]).wait()

    sem_o = sem_w + n_chunk
    wo32 = wo_hbm.bitcast(_U32)

    def wo_copy(j):
        return pltpu.make_async_copy(wo32.at[:, pl.ds(j * 128, 128)], wo.at[j], sems.at[sem_o + j])

    sem_f = sem_o + n_col
    ffn_copies = [pltpu.make_async_copy(a, b, sems.at[sem_f + i])
                  for i, (a, b) in enumerate(((wg_hbm, wg), (wu_hbm, wu), (wd_hbm, wd)))]

    x_copy(0).start()
    w_copy(0).start()
    for c in range(1, n_chunk):
        w_copy(c).start()
        if c < n_chunk - 1:
            x_copy(c).start()
    for cp in ffn_copies:
        cp.start()
    for j in range(n_col):
        wo_copy(j).start()

    def layernorm(r0, n):
        blk = 64
        for i in range(n // blk):
            rows = pl.ds(r0 + i * blk, blk)
            v = xb[rows, :].astype(_F32)
            mean = jnp.mean(v, axis=-1, keepdims=True)
            dev = v - mean
            var = jnp.mean(dev * dev, axis=-1, keepdims=True)
            den = _rnd(jnp.sqrt(_rnd(_rnd(var) + _LN_EPS)))
            y = _rnd(_rnd(v - _rnd(mean)) / den)
            xn[rows, :] = y
            gate[rows, :] = _silu(y)

    def retile(c):
        blk = 128
        for j in range(_CH // 2):
            for d0 in range(0, D, blk):
                u = stg[c, pl.ds(d0 * (_CH // 2) + j, blk, stride=_CH // 2), :]
                lo = pltpu.bitcast(u.astype(jnp.uint16), _U32)
                hi = pltpu.bitcast((u >> 16).astype(jnp.uint16), _U32)
                w[c * _CH + 2 * j, pl.ds(d0 // 2, blk // 2), :] = lo
                w[c * _CH + 2 * j + 1, pl.ds(d0 // 2, blk // 2), :] = hi

    def weights(ids):
        return pltpu.bitcast(jnp.concatenate([w[i] for i in ids], axis=1), _BF16)

    def bulk(c):
        for q in range(_CH // _G):
            ids = [c * _CH + q * _G + j for j in range(_G)]
            t = jnp.dot(xn[0:pre, :], weights(ids), preferred_element_type=_F32)
            for j, i in enumerate(ids):
                ring[i, ring_off:ring_rows, :] = t[:, j * dh:(j + 1) * dh]

    x_copy(0).wait()
    layernorm(0, pre)
    w_copy(0).wait()
    retile(0)

    def chunk_body(c, carry):
        w_wait_dyn(c + 1)
        x_copy_dyn(c).wait()
        bulk(c)
        retile(c + 1)
        layernorm(pl.multiple_of(pre + c * ln_rows, 64), ln_rows)
        return carry

    lax.fori_loop(0, n_chunk - 2, chunk_body, 0)

    w_copy(n_chunk - 1).wait()
    for cp in ffn_copies:
        cp.wait()

    wr = jnp.broadcast_to(wr_ref[...].astype(_F32).reshape(1, D), (8, D))
    r_all = lax.dot_general(wr, xn[...].astype(_BF16), _NT, preferred_element_type=_F32)
    sub = lax.broadcasted_iota(jnp.int32, (8, 128), 0)
    lane = lax.broadcasted_iota(jnp.int32, (8, 128), 1)
    vals, idxs = [], []
    for b in range(S // 1024):
        v = r_all[:, b * 1024:b * 1024 + 128]
        for t in range(1, 8):
            v = jnp.where(sub == t, r_all[:, b * 1024 + t * 128:b * 1024 + (t + 1) * 128], v)
        v = _rnd(v)
        vals.append(jnp.where(v != v, -jnp.inf, v))
        idxs.append((b * 1024 + sub * 128 + lane).astype(_F32))
    bulk(n_chunk - 2)
    retile(n_chunk - 1)

    sel_i, sel_x = [], []
    r_sel = jnp.zeros((_TOP_C, 128), _F32)
    for k in range(_TOP_C):
        m = functools.reduce(jnp.maximum, vals)
        m = jnp.max(jnp.max(m, axis=1, keepdims=True), axis=0, keepdims=True)
        cand = [jnp.where(v == m, i, float(S)) for v, i in zip(vals, idxs)]
        first = functools.reduce(jnp.minimum, cand)
        first = jnp.min(jnp.min(first, axis=1, keepdims=True), axis=0, keepdims=True)
        vals = [jnp.where(i == first, -jnp.inf, v) for v, i in zip(vals, idxs)]
        idxs = [jnp.where(i == first, float(S), i) for i in idxs]
        r_sel = jnp.where(sub == k, m, r_sel)
        tok = jnp.clip(first[0, 0].astype(jnp.int32), 0, S - 1)
        sel_i.append(tok)
        sel_x.append(xn[pl.ds(tok, 1), :])
    x_sel = jnp.concatenate(sel_x, axis=0)
    hg = _rnd(lax.dot_general(x_sel, wg[...], _NT, preferred_element_type=_F32))
    hu = _rnd(lax.dot_general(x_sel, wu[...], _NT, preferred_element_type=_F32))
    y = _rnd(jnp.dot(_rnd(_silu(hg)) * hu, wd[...], preferred_element_type=_F32))
    y = _rnd(y * _rnd(jax.nn.sigmoid(r_sel[:, 0:1])))
    g_sel = _silu(_rnd(x_sel + y))
    for k in range(_TOP_C):
        gate[pl.ds(sel_i[k], 1), :] = g_sel[k:k + 1, :]

    bulk(n_chunk - 1)

    for j in range(n_col):
        wo_copy(j).wait()

    qi = lax.broadcasted_iota(jnp.int32, (L, L), 0)
    ki = lax.broadcasted_iota(jnp.int32, (L, L), 1)
    mask = (qi >= seg) | (ki >= seg) | (qi >= ki)
    scale = dh ** -0.5

    def finish(s):
        rows = pl.ds(pl.multiple_of(s * seg, seg), seg)
        sg = _rnd(_rnd(sbuf[...]) * _rnd(gate[rows, :]))
        obuf[rows, :] = (xb[rows, :].astype(_F32) + sg).astype(_BF16)
        pltpu.make_async_copy(obuf.at[rows], out_hbm.at[rows], osem).start()

    def step(s, mem):
        @pl.when(s > 0)
        def _():
            finish(s - 1)

        xr = xn[pl.ds(pl.multiple_of(pre + s * xrows, 8), xrows), :]
        h = jnp.concatenate([xr, mem], axis=0)
        wpos = pl.ds(pl.multiple_of(lax.rem(s * xrows, ring_rows), 8), xrows)
        rpos = pl.ds(pl.multiple_of(lax.rem(s * seg + ring_off, ring_rows), 8), seg)
        xresult, presult, probs, heads_out = {}, {}, {}, {}
        acc = [None]

        def stage_a(g):
            ids = [m * heads + g * _G + j for m in range(3) for j in range(_G)]
            t = jnp.dot(h, weights(ids), preferred_element_type=_F32)
            for n, i in enumerate(ids):
                xresult[i] = t[:xrows, n * dh:(n + 1) * dh]
                presult[i] = t[xrows:, n * dh:(n + 1) * dh]

        def stage_w(g):
            for m in range(3):
                for j in range(_G):
                    i = m * heads + g * _G + j
                    ring[i, wpos, :] = xresult.pop(i)

        def rows_of(i):
            return jnp.concatenate([ring[i, rpos, :], presult[i]], axis=0)

        def stage_s(g):
            for j in range(_G):
                hd = g * _G + j
                k = rows_of(heads + hd).astype(_BF16)
                sc = lax.dot_general(rows_of(hd), k, _NT, preferred_element_type=_F32) * scale
                sc = jnp.where(mask, sc, -1000000000.0)
                e = jnp.exp(sc - jnp.max(sc, axis=-1, keepdims=True))
                probs[hd] = (e, 1.0 / jnp.sum(e, axis=-1, keepdims=True))

        def stage_p(g):
            outs = []
            for j in range(_G):
                hd = g * _G + j
                e, inv = probs[hd]
                v = rows_of(2 * heads + hd).astype(_BF16)
                outs.append(jnp.dot(e, v, preferred_element_type=_F32) * inv)
            heads_out[g] = jnp.concatenate(outs, axis=1)

        def stage_o(g):
            n = _G * dh // 2
            wt = jnp.concatenate([wo[j, g * n:(g + 1) * n, :] for j in range(n_col)], axis=1)
            t = jnp.dot(heads_out[g], pltpu.bitcast(wt, _BF16), preferred_element_type=_F32)
            acc[0] = t if acc[0] is None else acc[0] + t

        stages = {"A": stage_a, "W": stage_w, "S": stage_s, "P": stage_p, "O": stage_o}
        for name, g in _schedule(ng):
            stages[name](g)
        sbuf[...] = acc[0][:seg]
        return acc[0][seg:]

    lax.fori_loop(0, n_seg, step, mem0_ref[...].astype(_F32))
    finish(n_seg - 1)
    pltpu.make_async_copy(obuf, obuf, osem).wait()


@functools.partial(jax.jit, static_argnames=("A_seg_len",))
def pallas_recurrent_scan__memory_aug_recurrent_mem_tr__moe_arch_mod__prompt_kernel(
    A_x, A_mem0, A_Wq, A_Wk, A_Wv, A_Wo, A_seg_len,
    B_x, B_w_r, B_w_gate, B_w_up, B_w_down,
):
    del B_x
    B, S, D = A_x.shape
    _, H, Dh = A_Wq.shape
    M = A_mem0.shape[1]
    F = B_w_gate.shape[1]
    seg = int(A_seg_len)
    assert B == 1 and S % seg == 0 and Dh == 128 and D % 128 == 0 and H % _CH == 0
    xrows = seg - M
    pre = S - (S // seg) * xrows
    lcm = int(np.lcm(seg, xrows))
    ring_rows = -(-(pre + xrows) // lcm) * lcm
    n_chunk = 3 * H // _CH
    n_sem = (n_chunk - 1) + n_chunk + D // 128 + 3

    hbm = pl.BlockSpec(memory_space=pltpu.HBM)
    vmem = pl.BlockSpec(memory_space=pltpu.VMEM)
    out = pl.pallas_call(
        functools.partial(_kernel, seg=seg, n_mem=M, heads=H, dh=Dh),
        out_shape=jax.ShapeDtypeStruct((S, D), A_x.dtype),
        in_specs=[hbm, vmem, hbm, hbm, hbm, hbm, vmem, hbm, hbm, hbm],
        out_specs=hbm,
        scratch_shapes=[
            pltpu.VMEM((S, D), _BF16),
            pltpu.VMEM((S, D), _F32),
            pltpu.VMEM((S, D), _F32),
            pltpu.VMEM((n_chunk, D * _CH // 2, Dh), _U32),
            pltpu.VMEM((3 * H, D // 2, Dh), _U32),
            pltpu.VMEM((D // 128, H * Dh // 2, 128), _U32),
            pltpu.VMEM((3 * H, ring_rows, Dh), _F32),
            pltpu.VMEM((F, D), _BF16),
            pltpu.VMEM((F, D), _BF16),
            pltpu.VMEM((F, D), _BF16),
            pltpu.VMEM((seg, D), _F32),
            pltpu.VMEM((S, D), _BF16),
            pltpu.SemaphoreType.DMA((n_sem,)),
            pltpu.SemaphoreType.DMA(()),
        ],
        compiler_params=pltpu.CompilerParams(vmem_limit_bytes=112 * 1024 * 1024),
    )(
        A_x.reshape(S, D), A_mem0.reshape(M, D), A_Wq, A_Wk, A_Wv, A_Wo.reshape(H * Dh, D),
        B_w_r, B_w_gate.T, B_w_up.T, B_w_down,
    )
    return out.reshape(B, S, D)
```

```python
import functools

import jax
import jax.numpy as jnp
import numpy as np
from jax import lax
from jax.experimental import pallas as pl
from jax.experimental.pallas import tpu as pltpu

_F32 = jnp.float32
_BF16 = jnp.bfloat16
_U32 = jnp.uint32
_NT = (((1,), (1,)), ((), ()))

_TOP_C = 8
_G = 4
_CH = 16
_LN_EPS = 1e-05
_LN_BLK = 64
_BULK_ROWS = 128
_FFN_BLK = 128


def _rnd(v):
    return v.astype(_BF16).astype(_F32)


def _silu(v):
    half = 0.5 * v
    return half * jnp.tanh(half) + half


def _after(v, anchor):
    if anchor is None:
        return v
    keep = (pltpu.bitcast(anchor, jnp.int32) | 1) != 0
    keep = jnp.tile(keep, (v.shape[0] // 8, v.shape[1] // 128))
    return jnp.where(keep, v, jnp.zeros_like(v))


def _schedule(ng):
    toks = []
    for g in range(ng):
        toks.append(("A", g))
        if g >= 1:
            toks.append(("S", g - 1))
        if g >= 3:
            toks.append(("P", g - 3))
        toks.append(("W", g))
    tail = [[("S", ng - 1), ("P", ng - 3)], [("P", ng - 2)], [("P", ng - 1)]]
    o = 0
    for grp in tail:
        for _ in range(ng // 4):
            toks.append(("O", o))
            o += 1
        toks += grp
    while o < ng:
        toks.append(("O", o))
        o += 1
    return toks


def _kernel(x_hbm, mem0_hbm, wq_hbm, wk_hbm, wv_hbm, wo_hbm, wr_hbm, wg_hbm, wu_hbm, wd_hbm,
            out_hbm,
            xb, xn, xpre, xg, stg, w, wo, ring, wg, wu, wd, wr_ref, mem0_ref, sbuf, obuf, sems, osem,
            *, seg, n_mem, heads, dh):
    S, D = xb.shape
    n_seg = S // seg
    L = seg + n_mem
    xrows = seg - n_mem
    pre = S - n_seg * xrows
    ring_rows = ring.shape[1]
    ring_off = ring_rows - pre
    n_chunk = 3 * heads // _CH
    n_col = D // 128
    ln_rows = (S - pre) // 4
    ng = heads // _G

    x_parts = [(0, pre), (pre, ln_rows), (pre + ln_rows, S - pre - ln_rows)]
    srcs = [(x_hbm.at[pl.ds(r0, n)], xb.at[pl.ds(r0, n)]) for r0, n in x_parts]
    for c in range(n_chunk):
        src = (wq_hbm, wk_hbm, wv_hbm)[c // (heads // _CH)].bitcast(_U32)
        h2 = (c % (heads // _CH)) * (_CH // 2)
        srcs.append((src.at[:, pl.ds(h2, _CH // 2), :], stg.at[c].reshape(D, _CH // 2, dh)))
    wo32 = wo_hbm.bitcast(_U32)
    for j in range(n_col):
        srcs.append((wo32.at[:, pl.ds(j * 128, 128)], wo.at[j]))
    srcs += [(wg_hbm, wg), (wu_hbm, wu), (wd_hbm, wd), (wr_hbm, wr_ref), (mem0_hbm, mem0_ref)]
    copies = [pltpu.make_async_copy(a, b, sems.at[i]) for i, (a, b) in enumerate(srcs)]
    x_cp, copies = copies[:len(x_parts)], copies[len(x_parts):]
    w_cp, copies = copies[:n_chunk], copies[n_chunk:]
    wo_cp, copies = copies[:n_col], copies[n_col:]
    ffn_cp, small_cp = copies[:3], copies[3:]

    for cp in ([x_cp[0], w_cp[0]] + small_cp + [w_cp[1], x_cp[1], w_cp[2], w_cp[3], x_cp[2], w_cp[4]]
               + ffn_cp + [w_cp[5]] + wo_cp):
        cp.start()

    def layernorm(r0, anchor=None):
        rows = pl.ds(r0, _LN_BLK)
        v = xb[rows, :].astype(_F32)
        v = jnp.concatenate([_after(v[:, :128], anchor), v[:, 128:]], axis=1)
        mean = jnp.mean(v, axis=-1, keepdims=True)
        dev = v - mean
        var = jnp.mean(dev * dev, axis=-1, keepdims=True)
        den = _rnd(jnp.sqrt(_rnd(_rnd(var) + _LN_EPS)))
        y = (_rnd(v - _rnd(mean)) * (1.0 / den)).astype(_BF16)
        if r0 < pre:
            xpre[pl.ds(r0 // 2, _LN_BLK // 2), :] = pltpu.bitcast(y, _U32)
        xn[rows, :] = y.astype(_F32)
        xg[rows, :] = y.astype(_F32)

    def retile(pair, anchor=None):
        c, j = divmod(pair, _CH // 2)
        blk = 128
        for d0 in range(0, D, blk):
            u = stg[c, pl.ds(d0 * (_CH // 2) + j, blk, stride=_CH // 2), :]
            lo = pltpu.bitcast(u.astype(jnp.uint16), _U32)
            hi = pltpu.bitcast((u >> 16).astype(jnp.uint16), _U32)
            w[2 * pair, pl.ds(d0 // 2, blk // 2), :] = lo
            w[2 * pair + 1, pl.ds(d0 // 2, blk // 2), :] = hi

    def weights(ids):
        return pltpu.bitcast(jnp.concatenate([w[i] for i in ids], axis=1), _BF16)

    def bulk(grp, r0):
        ids = [grp * _G + j for j in range(_G)]
        lhs = pltpu.bitcast(xpre[pl.ds(r0 // 2, _BULK_ROWS // 2), :], _BF16)
        t = jnp.dot(lhs, weights(ids), preferred_element_type=_F32)
        for j, i in enumerate(ids):
            ring[i, pl.ds(ring_off + r0, _BULK_ROWS), :] = t[:, j * dh:(j + 1) * dh]
        return t[:8, :128]

    sub = lax.broadcasted_iota(jnp.int32, (8, 128), 0)
    lane = lax.broadcasted_iota(jnp.int32, (8, 128), 1)
    logits = {}
    routed = {}

    def router_tile(t, anchor=None):
        wr = jnp.broadcast_to(wr_ref[...].astype(_F32).reshape(1, D), (8, D))
        r = lax.dot_general(wr, xn[pl.ds(t * 128, 128), :].astype(_BF16), _NT,
                            preferred_element_type=_F32)
        b, row = divmod(t, 8)
        logits[b] = r if row == 0 else jnp.where(sub == row, r, logits[b])

    def top_c(anchor=None):
        vals, idxs = [], []
        for b in sorted(logits):
            v = _rnd(logits[b])
            vals.append(jnp.where(v != v, -jnp.inf, v))
            idxs.append((b * 1024 + sub * 128 + lane).astype(_F32))
        sel = []
        r_sel = jnp.zeros((_TOP_C, 128), _F32)
        for k in range(_TOP_C):
            m = functools.reduce(jnp.maximum, vals)
            m = jnp.max(jnp.max(m, axis=1, keepdims=True), axis=0, keepdims=True)
            cand = [jnp.where(v == m, i, float(S)) for v, i in zip(vals, idxs)]
            first = functools.reduce(jnp.minimum, cand)
            first = jnp.min(jnp.min(first, axis=1, keepdims=True), axis=0, keepdims=True)
            vals = [jnp.where(i == first, -jnp.inf, v) for v, i in zip(vals, idxs)]
            idxs = [jnp.where(i == first, float(S), i) for i in idxs]
            r_sel = jnp.where(sub == k, m, r_sel)
            sel.append(jnp.clip(first[0, 0].astype(jnp.int32), 0, S - 1))
        routed["sel"] = sel
        routed["r"] = r_sel[:, 0:1]
        routed["x"] = jnp.concatenate([xn[pl.ds(tok, 1), :] for tok in sel], axis=0)

    n_ffn = wg.shape[0]
    ffn_blocks = [(f0, min(_FFN_BLK, n_ffn - f0)) for f0 in range(0, n_ffn, _FFN_BLK)]

    def expert(n, anchor=None):
        if n > 0:
            f0, fn = ffn_blocks[n - 1]
            t = jnp.dot(routed.pop("h"), wd[pl.ds(f0, fn), :], preferred_element_type=_F32)
            routed["y"] = t if n == 1 else routed["y"] + t
        if n < len(ffn_blocks):
            f0, fn = ffn_blocks[n]
            hg = lax.dot_general(routed["x"], wg[pl.ds(f0, fn), :], _NT, preferred_element_type=_F32)
            hu = lax.dot_general(routed["x"], wu[pl.ds(f0, fn), :], _NT, preferred_element_type=_F32)
            routed["h"] = _rnd(_silu(_rnd(hg))) * _rnd(hu)
        else:
            y = _rnd(_rnd(routed["y"]) * _rnd(jax.nn.sigmoid(routed["r"])))
            rows = _rnd(routed["x"] + y)
            for k, tok in enumerate(routed["sel"]):
                xg[pl.ds(tok, 1), :] = rows[k:k + 1, :]

    per_grp = pre // _BULK_ROWS
    per_chunk = per_grp * (_CH // _G)
    n_slot = per_chunk * n_chunk
    waits = {per_chunk - per_grp: [w_cp[1], x_cp[1]] + small_cp,
             2 * per_chunk - per_grp: [w_cp[2], w_cp[3], x_cp[2]],
             4 * per_chunk - per_grp: [w_cp[4]] + ffn_cp,
             5 * per_chunk - per_grp: [w_cp[5]]}
    side = [[] for _ in range(n_slot)]

    def spread(tasks, first, last):
        for n, task in enumerate(tasks):
            side[first + n * (last - first + 1) // len(tasks)].append(task)

    def ln_tasks(part):
        r0, n = x_parts[part]
        return [functools.partial(layernorm, r) for r in range(r0, r0 + n, _LN_BLK)]

    def router_tasks(part):
        r0, n = x_parts[part]
        return [functools.partial(router_tile, t) for t in range(r0 // 128, (r0 + n) // 128)]

    for grp in range(1, n_slot // per_grp):
        for j in range(_G // 2):
            side[(grp - 1) * per_grp + j].append(functools.partial(retile, grp * (_G // 2) + j))
    b1, b2, b3, _ = sorted(waits)
    spread(ln_tasks(1), b1 + 1, b2 - 3)
    spread(router_tasks(0), b1 + 1, b2 - 3)
    spread(ln_tasks(2), b2 + 1, b3 - 8)
    spread(router_tasks(1), b2 + 1, b2 + 8)
    spread(router_tasks(2), b3 - 7, b3 - 1)
    side[b3].append(top_c)
    spread([functools.partial(expert, n) for n in range(len(ffn_blocks) + 1)], b3 + 8, n_slot - 4)

    x_cp[0].wait()
    for task in ln_tasks(0):
        task()
    w_cp[0].wait()
    for j in range(_G // 2):
        retile(j)
    for slot in range(n_slot):
        for cp in waits.get(slot, []):
            cp.wait()
        anchor = bulk(slot // per_grp, (slot % per_grp) * _BULK_ROWS)
        for task in side[slot]:
            task(anchor)

    for cp in wo_cp:
        cp.wait()

    qi = lax.broadcasted_iota(jnp.int32, (L, L), 0)
    ki = lax.broadcasted_iota(jnp.int32, (L, L), 1)
    mask = (qi >= seg) | (ki >= seg) | (qi >= ki)
    scale = dh ** -0.5

    def finish(s):
        rows = pl.ds(pl.multiple_of(s * seg, seg), seg)
        sg = _rnd(_rnd(sbuf[...]) * _rnd(_silu(xg[rows, :])))
        obuf[rows, :] = (xb[rows, :].astype(_F32) + sg).astype(_BF16)

    def send(s):
        rows = pl.ds(pl.multiple_of(s * seg, seg), seg)
        pltpu.make_async_copy(obuf.at[rows], out_hbm.at[rows], osem).start()

    def step(s, mem):
        finish(jnp.maximum(s - 1, 0))
        xr = xn[pl.ds(pl.multiple_of(pre + s * xrows, 8), xrows), :]
        h = jnp.concatenate([xr, mem], axis=0).astype(_BF16)
        wpos = pl.ds(pl.multiple_of(lax.rem(s * xrows, ring_rows), 8), xrows)
        rpos = pl.ds(pl.multiple_of(lax.rem(s * seg + ring_off, ring_rows), 8), seg)
        xresult, presult, probs, heads_out = {}, {}, {}, {}
        acc = [None]

        def stage_a(g):
            ids = [m * heads + g * _G + j for m in range(3) for j in range(_G)]
            t = jnp.dot(h, weights(ids), preferred_element_type=_F32)
            for n, i in enumerate(ids):
                xresult[i] = t[:xrows, n * dh:(n + 1) * dh]
                presult[i] = t[xrows:, n * dh:(n + 1) * dh]

        def stage_w(g):
            for m in range(3):
                for j in range(_G):
                    i = m * heads + g * _G + j
                    ring[i, wpos, :] = xresult.pop(i)

        def rows_of(i):
            return jnp.concatenate([ring[i, rpos, :], presult[i]], axis=0)

        def stage_s(g):
            for j in range(_G):
                hd = g * _G + j
                k = rows_of(heads + hd).astype(_BF16)
                sc = lax.dot_general(rows_of(hd), k, _NT, preferred_element_type=_F32) * scale
                sc = jnp.where(mask, sc, -1000000000.0)
                e = jnp.exp(sc - jnp.max(sc, axis=-1, keepdims=True))
                probs[hd] = (e, 1.0 / jnp.sum(e, axis=-1, keepdims=True))

        def stage_p(g):
            outs = []
            for j in range(_G):
                hd = g * _G + j
                e, inv = probs[hd]
                v = rows_of(2 * heads + hd).astype(_BF16)
                outs.append(jnp.dot(e, v, preferred_element_type=_F32) * inv)
            heads_out[g] = jnp.concatenate(outs, axis=1)

        def stage_o(g):
            n = _G * dh // 2
            wt = jnp.concatenate([wo[j, g * n:(g + 1) * n, :] for j in range(n_col)], axis=1)
            t = jnp.dot(heads_out[g], pltpu.bitcast(wt, _BF16), preferred_element_type=_F32)
            acc[0] = t if acc[0] is None else acc[0] + t

        stages = {"A": stage_a, "W": stage_w, "S": stage_s, "P": stage_p, "O": stage_o}
        for name, g in _schedule(ng):
            stages[name](g)
        sbuf[...] = acc[0][:seg]

        @pl.when(s > 0)
        def _():
            send(s - 1)

        return acc[0][seg:]

    sbuf[...] = jnp.zeros(sbuf.shape, _F32)
    lax.fori_loop(0, n_seg, step, mem0_ref[...].astype(_F32))
    finish(n_seg - 1)
    send(n_seg - 1)
    pltpu.make_async_copy(obuf, obuf, osem).wait()


@functools.partial(jax.jit, static_argnames=("A_seg_len",))
def pallas_recurrent_scan__memory_aug_recurrent_mem_tr__moe_arch_mod__prompt_kernel(
    A_x, A_mem0, A_Wq, A_Wk, A_Wv, A_Wo, A_seg_len,
    B_x, B_w_r, B_w_gate, B_w_up, B_w_down,
):
    del B_x
    B, S, D = A_x.shape
    _, H, Dh = A_Wq.shape
    M = A_mem0.shape[1]
    F = B_w_gate.shape[1]
    seg = int(A_seg_len)
    assert B == 1 and S % seg == 0 and Dh == 128 and D % 128 == 0 and H % _CH == 0
    xrows = seg - M
    pre = S - (S // seg) * xrows
    lcm = int(np.lcm(seg, xrows))
    ring_rows = -(-(pre + xrows) // lcm) * lcm
    n_chunk = 3 * H // _CH
    n_sem = 3 + n_chunk + D // 128 + 5

    hbm = pl.BlockSpec(memory_space=pltpu.HBM)
    out = pl.pallas_call(
        functools.partial(_kernel, seg=seg, n_mem=M, heads=H, dh=Dh),
        out_shape=jax.ShapeDtypeStruct((S, D), A_x.dtype),
        in_specs=[hbm] * 10,
        out_specs=hbm,
        scratch_shapes=[
            pltpu.VMEM((S, D), _BF16),
            pltpu.VMEM((S, D), _F32),
            pltpu.VMEM((pre // 2, D), _U32),
            pltpu.VMEM((S, D), _F32),
            pltpu.VMEM((n_chunk, D * _CH // 2, Dh), _U32),
            pltpu.VMEM((3 * H, D // 2, Dh), _U32),
            pltpu.VMEM((D // 128, H * Dh // 2, 128), _U32),
            pltpu.VMEM((3 * H, ring_rows, Dh), _F32),
            pltpu.VMEM((F, D), _BF16),
            pltpu.VMEM((F, D), _BF16),
            pltpu.VMEM((F, D), _BF16),
            pltpu.VMEM((D,), _BF16),
            pltpu.VMEM((M, D), _BF16),
            pltpu.VMEM((seg, D), _F32),
            pltpu.VMEM((S, D), _BF16),
            pltpu.SemaphoreType.DMA((n_sem,)),
            pltpu.SemaphoreType.DMA(()),
        ],
        compiler_params=pltpu.CompilerParams(vmem_limit_bytes=112 * 1024 * 1024),
    )(
        A_x.reshape(S, D), A_mem0.reshape(M, D), A_Wq, A_Wk, A_Wv, A_Wo.reshape(H * Dh, D),
        B_w_r, B_w_gate.T, B_w_up.T, B_w_down,
    )
    return out.reshape(B, S, D)
```

```python
import functools

import jax
import jax.numpy as jnp
import numpy as np
from jax import lax
from jax.experimental import pallas as pl
from jax.experimental.pallas import tpu as pltpu

_F32 = jnp.float32
_BF16 = jnp.bfloat16
_U32 = jnp.uint32
_NT = (((1,), (1,)), ((), ()))

_TOP_C = 8
_G = 4
_CH = 16
_LN_EPS = 1e-05
_LN_BLK = 64
_BULK_ROWS = 128
_UNROLL = 4
_FFN_BLK = 128


def _rnd(v):
    return v.astype(_BF16).astype(_F32)


def _silu(v):
    half = 0.5 * v
    return half * jnp.tanh(half) + half


def _after(v, anchor):
    if anchor is None:
        return v
    keep = (pltpu.bitcast(anchor, jnp.int32) | 1) != 0
    keep = jnp.tile(keep, (v.shape[0] // 8, v.shape[1] // 128))
    return jnp.where(keep, v, jnp.zeros_like(v))


def _schedule(ng):
    toks = []
    for g in range(ng):
        toks.append(("A", g))
        if g >= 1:
            toks.append(("S", g - 1))
        if g >= 3:
            toks.append(("P", g - 3))
        toks.append(("W", g))
    tail = [[("S", ng - 1), ("P", ng - 3)], [("P", ng - 2)], [("P", ng - 1)]]
    o = 0
    for grp in tail:
        for _ in range(ng // 4):
            toks.append(("O", o))
            o += 1
        toks += grp
    while o < ng:
        toks.append(("O", o))
        o += 1
    return toks


def _kernel(x_hbm, mem0_hbm, wq_hbm, wk_hbm, wv_hbm, wo_hbm, wr_hbm, wg_hbm, wu_hbm, wd_hbm,
            out_hbm,
            xb, xn, xpre, xg, stg, w, wo, ring, wg, wu, wd, wr_ref, mem0_ref, sbuf, obuf, sems, osem,
            *, seg, n_mem, heads, dh):
    S, D = xb.shape
    n_seg = S // seg
    L = seg + n_mem
    xrows = seg - n_mem
    pre = S - n_seg * xrows
    ring_rows = ring.shape[1]
    ring_off = ring_rows - pre
    n_chunk = 3 * heads // _CH
    n_col = D // 128
    ln_rows = (S - pre) // 4
    ng = heads // _G

    x_parts = [(0, pre), (pre, ln_rows), (pre + ln_rows, S - pre - ln_rows)]
    srcs = [(x_hbm.at[pl.ds(r0, n)], xb.at[pl.ds(r0, n)]) for r0, n in x_parts]
    for c in range(n_chunk):
        src = (wq_hbm, wk_hbm, wv_hbm)[c // (heads // _CH)].bitcast(_U32)
        h2 = (c % (heads // _CH)) * (_CH // 2)
        srcs.append((src.at[:, pl.ds(h2, _CH // 2), :], stg.at[c].reshape(D, _CH // 2, dh)))
    wo32 = wo_hbm.bitcast(_U32)
    for j in range(n_col):
        srcs.append((wo32.at[:, pl.ds(j * 128, 128)], wo.at[j]))
    srcs += [(wg_hbm, wg), (wu_hbm, wu), (wd_hbm, wd), (wr_hbm, wr_ref), (mem0_hbm, mem0_ref)]
    copies = [pltpu.make_async_copy(a, b, sems.at[i]) for i, (a, b) in enumerate(srcs)]
    x_cp, copies = copies[:len(x_parts)], copies[len(x_parts):]
    w_cp, copies = copies[:n_chunk], copies[n_chunk:]
    wo_cp, copies = copies[:n_col], copies[n_col:]
    ffn_cp, small_cp = copies[:3], copies[3:]

    for cp in ([x_cp[0], w_cp[0]] + small_cp + [w_cp[1], x_cp[1], w_cp[2], w_cp[3], x_cp[2], w_cp[4]]
               + ffn_cp + [w_cp[5]] + wo_cp):
        cp.start()

    def layernorm(r0, anchor=None):
        rows = pl.ds(r0, _LN_BLK)
        v = xb[rows, :].astype(_F32)
        v = jnp.concatenate([_after(v[:, :128], anchor), v[:, 128:]], axis=1)
        mean = jnp.mean(v, axis=-1, keepdims=True)
        dev = v - mean
        var = jnp.mean(dev * dev, axis=-1, keepdims=True)
        den = _rnd(jnp.sqrt(_rnd(_rnd(var) + _LN_EPS)))
        y = (_rnd(v - _rnd(mean)) * (1.0 / den)).astype(_BF16)
        if r0 < pre:
            xpre[pl.ds(r0 // 2, _LN_BLK // 2), :] = pltpu.bitcast(y, _U32)
        xn[rows, :] = y.astype(_F32)
        xg[rows, :] = y.astype(_F32)

    def retile(pair, anchor=None):
        c, j = divmod(pair, _CH // 2)
        blk = 128
        for d0 in range(0, D, blk):
            u = stg[c, pl.ds(d0 * (_CH // 2) + j, blk, stride=_CH // 2), :]
            lo = pltpu.bitcast(u.astype(jnp.uint16), _U32)
            hi = pltpu.bitcast((u >> 16).astype(jnp.uint16), _U32)
            w[2 * pair, pl.ds(d0 // 2, blk // 2), :] = lo
            w[2 * pair + 1, pl.ds(d0 // 2, blk // 2), :] = hi

    def weights(ids):
        return pltpu.bitcast(jnp.concatenate([w[i] for i in ids], axis=1), _BF16)

    def bulk(grp, r0):
        ids = [grp * _G + j for j in range(_G)]
        lhs = pltpu.bitcast(xpre[pl.ds(r0 // 2, _BULK_ROWS // 2), :], _BF16)
        t = jnp.dot(lhs, weights(ids), preferred_element_type=_F32)
        for j, i in enumerate(ids):
            ring[i, pl.ds(ring_off + r0, _BULK_ROWS), :] = t[:, j * dh:(j + 1) * dh]
        return t[:8, :128]

    sub = lax.broadcasted_iota(jnp.int32, (8, 128), 0)
    lane = lax.broadcasted_iota(jnp.int32, (8, 128), 1)
    logits = {}
    routed = {}

    def router_tile(t, anchor=None):
        wr = jnp.broadcast_to(wr_ref[...].astype(_F32).reshape(1, D), (8, D))
        r = lax.dot_general(wr, xn[pl.ds(t * 128, 128), :].astype(_BF16), _NT,
                            preferred_element_type=_F32)
        b, row = divmod(t, 8)
        logits[b] = r if row == 0 else jnp.where(sub == row, r, logits[b])

    def top_c(anchor=None):
        vals, idxs = [], []
        for b in sorted(logits):
            v = _rnd(logits[b])
            vals.append(jnp.where(v != v, -jnp.inf, v))
            idxs.append((b * 1024 + sub * 128 + lane).astype(_F32))
        sel = []
        r_sel = jnp.zeros((_TOP_C, 128), _F32)
        for k in range(_TOP_C):
            m = functools.reduce(jnp.maximum, vals)
            m = jnp.max(jnp.max(m, axis=1, keepdims=True), axis=0, keepdims=True)
            cand = [jnp.where(v == m, i, float(S)) for v, i in zip(vals, idxs)]
            first = functools.reduce(jnp.minimum, cand)
            first = jnp.min(jnp.min(first, axis=1, keepdims=True), axis=0, keepdims=True)
            vals = [jnp.where(i == first, -jnp.inf, v) for v, i in zip(vals, idxs)]
            idxs = [jnp.where(i == first, float(S), i) for i in idxs]
            r_sel = jnp.where(sub == k, m, r_sel)
            sel.append(jnp.clip(first[0, 0].astype(jnp.int32), 0, S - 1))
        routed["sel"] = sel
        routed["r"] = r_sel[:, 0:1]
        routed["x"] = jnp.concatenate([xn[pl.ds(tok, 1), :] for tok in sel], axis=0)

    n_ffn = wg.shape[0]
    ffn_blocks = [(f0, min(_FFN_BLK, n_ffn - f0)) for f0 in range(0, n_ffn, _FFN_BLK)]

    def expert(n, anchor=None):
        if n > 0:
            f0, fn = ffn_blocks[n - 1]
            t = jnp.dot(routed.pop("h"), wd[pl.ds(f0, fn), :], preferred_element_type=_F32)
            routed["y"] = t if n == 1 else routed["y"] + t
        if n < len(ffn_blocks):
            f0, fn = ffn_blocks[n]
            hg = lax.dot_general(routed["x"], wg[pl.ds(f0, fn), :], _NT, preferred_element_type=_F32)
            hu = lax.dot_general(routed["x"], wu[pl.ds(f0, fn), :], _NT, preferred_element_type=_F32)
            routed["h"] = _rnd(_silu(_rnd(hg))) * _rnd(hu)
        else:
            y = _rnd(_rnd(routed["y"]) * _rnd(jax.nn.sigmoid(routed["r"])))
            rows = _rnd(routed["x"] + y)
            for k, tok in enumerate(routed["sel"]):
                xg[pl.ds(tok, 1), :] = rows[k:k + 1, :]

    per_grp = pre // _BULK_ROWS
    per_chunk = per_grp * (_CH // _G)
    n_slot = per_chunk * n_chunk
    waits = {per_chunk - per_grp: [w_cp[1], x_cp[1]] + small_cp,
             2 * per_chunk - per_grp: [w_cp[2], w_cp[3], x_cp[2]],
             4 * per_chunk - per_grp: [w_cp[4]] + ffn_cp,
             5 * per_chunk - per_grp: [w_cp[5]]}
    side = [[] for _ in range(n_slot)]

    def spread(tasks, first, last):
        for n, task in enumerate(tasks):
            side[first + n * (last - first + 1) // len(tasks)].append(task)

    def ln_tasks(part):
        r0, n = x_parts[part]
        return [functools.partial(layernorm, r) for r in range(r0, r0 + n, _LN_BLK)]

    def router_tasks(part):
        r0, n = x_parts[part]
        return [functools.partial(router_tile, t) for t in range(r0 // 128, (r0 + n) // 128)]

    for grp in range(1, n_slot // per_grp):
        for j in range(_G // 2):
            side[(grp - 1) * per_grp + j].append(functools.partial(retile, grp * (_G // 2) + j))
    b1, b2, b3, _ = sorted(waits)
    spread(ln_tasks(1), b1 + 1, b2 - 3)
    spread(router_tasks(0), b1 + 1, b2 - 3)
    spread(ln_tasks(2), b2 + 1, b3 - 8)
    spread(router_tasks(1), b2 + 1, b2 + 8)
    spread(router_tasks(2), b3 - 7, b3 - 1)
    side[b3].append(top_c)
    spread([functools.partial(expert, n) for n in range(len(ffn_blocks) + 1)], b3 + 8, n_slot - 4)

    x_cp[0].wait()
    for task in ln_tasks(0):
        task()
    w_cp[0].wait()
    for j in range(_G // 2):
        retile(j)
    for slot in range(n_slot):
        for cp in waits.get(slot, []):
            cp.wait()
        anchor = bulk(slot // per_grp, (slot % per_grp) * _BULK_ROWS)
        for task in side[slot]:
            task(anchor)

    for cp in wo_cp:
        cp.wait()

    qi = lax.broadcasted_iota(jnp.int32, (L, L), 0)
    ki = lax.broadcasted_iota(jnp.int32, (L, L), 1)
    mask = (qi >= seg) | (ki >= seg) | (qi >= ki)
    scale = dh ** -0.5

    def finish(s):
        rows = pl.ds(pl.multiple_of(s * seg, seg), seg)
        sg = _rnd(_rnd(sbuf[...]) * _rnd(_silu(xg[rows, :])))
        obuf[rows, :] = (xb[rows, :].astype(_F32) + sg).astype(_BF16)

    def send(it):
        rows = pl.ds(pl.multiple_of(it * (_UNROLL * seg), _UNROLL * seg), _UNROLL * seg)
        pltpu.make_async_copy(obuf.at[rows], out_hbm.at[rows], osem).start()

    def step(s, mem):
        finish(jnp.maximum(s - 1, 0))
        xr = xn[pl.ds(pl.multiple_of(pre + s * xrows, 8), xrows), :]
        h = jnp.concatenate([xr, mem], axis=0).astype(_BF16)
        wpos = pl.ds(pl.multiple_of(lax.rem(s * xrows, ring_rows), 8), xrows)
        rpos = pl.ds(pl.multiple_of(lax.rem(s * seg + ring_off, ring_rows), 8), seg)
        xresult, presult, probs, heads_out = {}, {}, {}, {}
        acc = [None]

        def stage_a(g):
            ids = [m * heads + g * _G + j for m in range(3) for j in range(_G)]
            t = jnp.dot(h, weights(ids), preferred_element_type=_F32)
            for n, i in enumerate(ids):
                xresult[i] = t[:xrows, n * dh:(n + 1) * dh]
                presult[i] = t[xrows:, n * dh:(n + 1) * dh]

        def stage_w(g):
            for m in range(3):
                for j in range(_G):
                    i = m * heads + g * _G + j
                    ring[i, wpos, :] = xresult.pop(i)

        def rows_of(i):
            return jnp.concatenate([ring[i, rpos, :], presult[i]], axis=0)

        def stage_s(g):
            for j in range(_G):
                hd = g * _G + j
                k = rows_of(heads + hd).astype(_BF16)
                sc = lax.dot_general(rows_of(hd), k, _NT, preferred_element_type=_F32) * scale
                sc = jnp.where(mask, sc, -1000000000.0)
                e = jnp.exp(sc - jnp.max(sc, axis=-1, keepdims=True))
                probs[hd] = (e, 1.0 / jnp.sum(e, axis=-1, keepdims=True))

        def stage_p(g):
            outs = []
            for j in range(_G):
                hd = g * _G + j
                e, inv = probs[hd]
                v = rows_of(2 * heads + hd).astype(_BF16)
                outs.append(jnp.dot(e, v, preferred_element_type=_F32) * inv)
            heads_out[g] = jnp.concatenate(outs, axis=1)

        def stage_o(g):
            n = _G * dh // 2
            wt = jnp.concatenate([wo[j, g * n:(g + 1) * n, :] for j in range(n_col)], axis=1)
            t = jnp.dot(heads_out[g], pltpu.bitcast(wt, _BF16), preferred_element_type=_F32)
            acc[0] = t if acc[0] is None else acc[0] + t

        stages = {"A": stage_a, "W": stage_w, "S": stage_s, "P": stage_p, "O": stage_o}
        for name, g in _schedule(ng):
            stages[name](g)
        sbuf[...] = acc[0][:seg]
        return acc[0][seg:]

    def steps(it, mem):
        for u in range(_UNROLL):
            mem = step(it * _UNROLL + u, mem)

        @pl.when(it > 0)
        def _():
            send(it - 1)

        return mem

    sbuf[...] = jnp.zeros(sbuf.shape, _F32)
    lax.fori_loop(0, n_seg // _UNROLL, steps, mem0_ref[...].astype(_F32))
    finish(n_seg - 1)
    send(n_seg // _UNROLL - 1)
    pltpu.make_async_copy(obuf, obuf, osem).wait()


@functools.partial(jax.jit, static_argnames=("A_seg_len",))
def pallas_recurrent_scan__memory_aug_recurrent_mem_tr__moe_arch_mod__prompt_kernel(
    A_x, A_mem0, A_Wq, A_Wk, A_Wv, A_Wo, A_seg_len,
    B_x, B_w_r, B_w_gate, B_w_up, B_w_down,
):
    del B_x
    B, S, D = A_x.shape
    _, H, Dh = A_Wq.shape
    M = A_mem0.shape[1]
    F = B_w_gate.shape[1]
    seg = int(A_seg_len)
    assert B == 1 and S % seg == 0 and Dh == 128 and D % 128 == 0 and H % _CH == 0
    xrows = seg - M
    pre = S - (S // seg) * xrows
    lcm = int(np.lcm(seg, xrows))
    ring_rows = -(-(pre + xrows) // lcm) * lcm
    n_chunk = 3 * H // _CH
    n_sem = 3 + n_chunk + D // 128 + 5

    hbm = pl.BlockSpec(memory_space=pltpu.HBM)
    out = pl.pallas_call(
        functools.partial(_kernel, seg=seg, n_mem=M, heads=H, dh=Dh),
        out_shape=jax.ShapeDtypeStruct((S, D), A_x.dtype),
        in_specs=[hbm] * 10,
        out_specs=hbm,
        scratch_shapes=[
            pltpu.VMEM((S, D), _BF16),
            pltpu.VMEM((S, D), _F32),
            pltpu.VMEM((pre // 2, D), _U32),
            pltpu.VMEM((S, D), _F32),
            pltpu.VMEM((n_chunk, D * _CH // 2, Dh), _U32),
            pltpu.VMEM((3 * H, D // 2, Dh), _U32),
            pltpu.VMEM((D // 128, H * Dh // 2, 128), _U32),
            pltpu.VMEM((3 * H, ring_rows, Dh), _F32),
            pltpu.VMEM((F, D), _BF16),
            pltpu.VMEM((F, D), _BF16),
            pltpu.VMEM((F, D), _BF16),
            pltpu.VMEM((D,), _BF16),
            pltpu.VMEM((M, D), _BF16),
            pltpu.VMEM((seg, D), _F32),
            pltpu.VMEM((S, D), _BF16),
            pltpu.SemaphoreType.DMA((n_sem,)),
            pltpu.SemaphoreType.DMA(()),
        ],
        compiler_params=pltpu.CompilerParams(vmem_limit_bytes=112 * 1024 * 1024),
    )(
        A_x.reshape(S, D), A_mem0.reshape(M, D), A_Wq, A_Wk, A_Wv, A_Wo.reshape(H * Dh, D),
        B_w_r, B_w_gate.T, B_w_up.T, B_w_down,
    )
    return out.reshape(B, S, D)
```

```python
import functools

import jax
import jax.numpy as jnp
import numpy as np
from jax import lax
from jax.experimental import pallas as pl
from jax.experimental.pallas import tpu as pltpu

_F32 = jnp.float32
_BF16 = jnp.bfloat16
_U32 = jnp.uint32
_NT = (((1,), (1,)), ((), ()))

_TOP_C = 8
_G = 4
_CH = 16
_LN_EPS = 1e-05
_LN_BLK = 64
_BULK_ROWS = 128
_UNROLL = 4
_D_SPLIT = 256
_FFN_BLK = 128


def _rnd(v):
    return v.astype(_BF16).astype(_F32)


def _silu(v):
    half = 0.5 * v
    return half * jnp.tanh(half) + half


def _after(v, anchor):
    if anchor is None:
        return v
    keep = (pltpu.bitcast(anchor, jnp.int32) | 1) != 0
    keep = jnp.tile(keep, (v.shape[0] // 8, v.shape[1] // 128))
    return jnp.where(keep, v, jnp.zeros_like(v))


def _schedule(ng):
    toks = []
    for g in range(ng):
        toks.append(("A", g))
        if g >= 1:
            toks.append(("S", g - 1))
        if g >= 3:
            toks.append(("P", g - 3))
        toks.append(("W", g))
    tail = [[("S", ng - 1), ("P", ng - 3)], [("P", ng - 2)], [("P", ng - 1)]]
    o = 0
    for grp in tail:
        for _ in range(ng // 4):
            toks.append(("O", o))
            o += 1
        toks += grp
    while o < ng:
        toks.append(("O", o))
        o += 1
    return toks


def _kernel(x_hbm, mem0_hbm, wq_hbm, wk_hbm, wv_hbm, wo_hbm, wr_hbm, wg_hbm, wu_hbm, wd_hbm,
            out_hbm,
            xb, xn, xpre, xg, stg, w, wo, ring, wg, wu, wd, wr_ref, mem0_ref, sbuf, obuf, sems, osem,
            *, seg, n_mem, heads, dh):
    S, D = xb.shape
    n_seg = S // seg
    L = seg + n_mem
    xrows = seg - n_mem
    pre = S - n_seg * xrows
    ring_rows = ring.shape[1]
    ring_off = ring_rows - pre
    n_chunk = 3 * heads // _CH
    n_col = D // 128
    ln_rows = (S - pre) // 4
    ng = heads // _G

    x_parts = [(0, pre), (pre, ln_rows), (pre + ln_rows, S - pre - ln_rows)]
    srcs = [(x_hbm.at[pl.ds(r0, n)], xb.at[pl.ds(r0, n)]) for r0, n in x_parts]
    for c, d0, d1 in [(0, 0, _D_SPLIT), (0, _D_SPLIT, D)] + [(c, 0, D) for c in range(1, n_chunk)]:
        src = (wq_hbm, wk_hbm, wv_hbm)[c // (heads // _CH)].bitcast(_U32)
        h2 = (c % (heads // _CH)) * (_CH // 2)
        srcs.append((src.at[pl.ds(d0, d1 - d0), pl.ds(h2, _CH // 2), :],
                     stg.at[c].reshape(D, _CH // 2, dh).at[pl.ds(d0, d1 - d0)]))
    wo32 = wo_hbm.bitcast(_U32)
    for j in range(n_col):
        srcs.append((wo32.at[:, pl.ds(j * 128, 128)], wo.at[j]))
    srcs += [(wg_hbm, wg), (wu_hbm, wu), (wd_hbm, wd), (wr_hbm, wr_ref), (mem0_hbm, mem0_ref)]
    copies = [pltpu.make_async_copy(a, b, sems.at[i]) for i, (a, b) in enumerate(srcs)]
    x_cp, copies = copies[:len(x_parts)], copies[len(x_parts):]
    w_first, w_cp, copies = copies[0], copies[1:n_chunk + 1], copies[n_chunk + 1:]
    wo_cp, copies = copies[:n_col], copies[n_col:]
    ffn_cp, small_cp = copies[:3], copies[3:]

    for cp in ([x_cp[0], w_first, w_cp[0]] + small_cp + [w_cp[1], x_cp[1], w_cp[2], x_cp[2], w_cp[3], w_cp[4]]
               + ffn_cp + [w_cp[5]] + wo_cp):
        cp.start()

    def layernorm(r0, anchor=None):
        rows = pl.ds(r0, _LN_BLK)
        v = xb[rows, :].astype(_F32)
        v = jnp.concatenate([_after(v[:, :128], anchor), v[:, 128:]], axis=1)
        mean = jnp.mean(v, axis=-1, keepdims=True)
        dev = v - mean
        var = jnp.mean(dev * dev, axis=-1, keepdims=True)
        den = _rnd(jnp.sqrt(_rnd(_rnd(var) + _LN_EPS)))
        y = (_rnd(v - _rnd(mean)) * (1.0 / den)).astype(_BF16)
        if r0 < pre:
            xpre[pl.ds(r0 // 2, _LN_BLK // 2), :] = pltpu.bitcast(y, _U32)
        xn[rows, :] = y.astype(_F32)
        xg[rows, :] = y.astype(_F32)

    def retile(pair, anchor=None, d_lo=0, d_hi=D):
        c, j = divmod(pair, _CH // 2)
        blk = 128
        for d0 in range(d_lo, d_hi, blk):
            u = stg[c, pl.ds(d0 * (_CH // 2) + j, blk, stride=_CH // 2), :]
            lo = pltpu.bitcast(u.astype(jnp.uint16), _U32)
            hi = pltpu.bitcast((u >> 16).astype(jnp.uint16), _U32)
            w[2 * pair, pl.ds(d0 // 2, blk // 2), :] = lo
            w[2 * pair + 1, pl.ds(d0 // 2, blk // 2), :] = hi

    def weights(ids, d_lo=0, d_hi=D):
        rows = pl.ds(d_lo // 2, (d_hi - d_lo) // 2)
        return pltpu.bitcast(jnp.concatenate([w[i, rows, :] for i in ids], axis=1), _BF16)

    def bulk(grp, r0, d_lo=0, d_hi=D):
        ids = [grp * _G + j for j in range(_G)]
        lhs = pltpu.bitcast(xpre[pl.ds(r0 // 2, _BULK_ROWS // 2), d_lo:d_hi], _BF16)
        t = jnp.dot(lhs, weights(ids, d_lo, d_hi), preferred_element_type=_F32)
        rows = pl.ds(ring_off + r0, _BULK_ROWS)
        for j, i in enumerate(ids):
            part = t[:, j * dh:(j + 1) * dh]
            ring[i, rows, :] = part if d_lo == 0 else ring[i, rows, :] + part
        return t[:8, :128]

    sub = lax.broadcasted_iota(jnp.int32, (8, 128), 0)
    lane = lax.broadcasted_iota(jnp.int32, (8, 128), 1)
    logits = {}
    routed = {}

    def router_tile(t, anchor=None):
        wr = jnp.broadcast_to(wr_ref[...].astype(_F32).reshape(1, D), (8, D))
        r = lax.dot_general(wr, xn[pl.ds(t * 128, 128), :].astype(_BF16), _NT,
                            preferred_element_type=_F32)
        b, row = divmod(t, 8)
        logits[b] = r if row == 0 else jnp.where(sub == row, r, logits[b])

    def top_c(anchor=None):
        vals, idxs = [], []
        for b in sorted(logits):
            v = _rnd(logits[b])
            vals.append(jnp.where(v != v, -jnp.inf, v))
            idxs.append((b * 1024 + sub * 128 + lane).astype(_F32))
        sel = []
        r_sel = jnp.zeros((_TOP_C, 128), _F32)
        for k in range(_TOP_C):
            m = functools.reduce(jnp.maximum, vals)
            m = jnp.max(jnp.max(m, axis=1, keepdims=True), axis=0, keepdims=True)
            cand = [jnp.where(v == m, i, float(S)) for v, i in zip(vals, idxs)]
            first = functools.reduce(jnp.minimum, cand)
            first = jnp.min(jnp.min(first, axis=1, keepdims=True), axis=0, keepdims=True)
            vals = [jnp.where(i == first, -jnp.inf, v) for v, i in zip(vals, idxs)]
            idxs = [jnp.where(i == first, float(S), i) for i in idxs]
            r_sel = jnp.where(sub == k, m, r_sel)
            sel.append(jnp.clip(first[0, 0].astype(jnp.int32), 0, S - 1))
        routed["sel"] = sel
        routed["r"] = r_sel[:, 0:1]
        routed["x"] = jnp.concatenate([xn[pl.ds(tok, 1), :] for tok in sel], axis=0)

    n_ffn = wg.shape[0]
    ffn_blocks = [(f0, min(_FFN_BLK, n_ffn - f0)) for f0 in range(0, n_ffn, _FFN_BLK)]

    def expert(n, anchor=None):
        if n > 0:
            f0, fn = ffn_blocks[n - 1]
            t = jnp.dot(routed.pop("h"), wd[pl.ds(f0, fn), :], preferred_element_type=_F32)
            routed["y"] = t if n == 1 else routed["y"] + t
        if n < len(ffn_blocks):
            f0, fn = ffn_blocks[n]
            hg = lax.dot_general(routed["x"], wg[pl.ds(f0, fn), :], _NT, preferred_element_type=_F32)
            hu = lax.dot_general(routed["x"], wu[pl.ds(f0, fn), :], _NT, preferred_element_type=_F32)
            routed["h"] = _rnd(_silu(_rnd(hg))) * _rnd(hu)
        else:
            y = _rnd(_rnd(routed["y"]) * _rnd(jax.nn.sigmoid(routed["r"])))
            rows = _rnd(routed["x"] + y)
            for k, tok in enumerate(routed["sel"]):
                xg[pl.ds(tok, 1), :] = rows[k:k + 1, :]

    per_grp = pre // _BULK_ROWS
    per_chunk = per_grp * (_CH // _G)
    n_slot = per_chunk * n_chunk
    waits = {per_chunk - per_grp: [w_cp[1], x_cp[1]] + small_cp,
             2 * per_chunk - per_grp: [w_cp[2], x_cp[2]],
             3 * per_chunk - per_grp: [w_cp[3], w_cp[4]],
             5 * per_chunk - per_grp: [w_cp[5]] + ffn_cp}
    side = [[] for _ in range(n_slot)]

    def spread(tasks, first, last):
        for n, task in enumerate(tasks):
            side[first + n * (last - first + 1) // len(tasks)].append(task)

    def ln_tasks(part):
        r0, n = x_parts[part]
        return [functools.partial(layernorm, r) for r in range(r0, r0 + n, _LN_BLK)]

    def router_tasks(part):
        r0, n = x_parts[part]
        return [functools.partial(router_tile, t) for t in range(r0 // 128, (r0 + n) // 128)]

    for grp in range(1, n_slot // per_grp):
        for j in range(_G // 2):
            side[(grp - 1) * per_grp + j].append(functools.partial(
                retile, grp * (_G // 2) + j, d_lo=_D_SPLIT if grp < _CH // _G else 0))
    b1, b2, b3, b4 = sorted(waits)
    late_ln = ln_tasks(2)
    spread(ln_tasks(1), b1 + 1, b2 - 3)
    spread(router_tasks(0), b1 + 1, b2 - 3)
    spread(late_ln[:len(late_ln) // 2], b2 + 1, b3 - 3)
    spread(router_tasks(1), b2 + 1, b3 - 3)
    spread(late_ln[len(late_ln) // 2:], b3 + 1, b3 + 12)
    spread(router_tasks(2), b3 + 8, b4 - 12)
    side[b4 - 10].append(top_c)
    spread([functools.partial(expert, n) for n in range(len(ffn_blocks) + 1)], b4 + 1, n_slot - 3)

    x_cp[0].wait()
    for task in ln_tasks(0):
        task()
    w_first.wait()
    for pair in range(_CH // 2):
        retile(pair, d_hi=_D_SPLIT)
    for slot in range(per_chunk):
        bulk(slot // per_grp, (slot % per_grp) * _BULK_ROWS, d_hi=_D_SPLIT)
    w_cp[0].wait()
    for j in range(_G // 2):
        retile(j, d_lo=_D_SPLIT)
    for slot in range(n_slot):
        for cp in waits.get(slot, []):
            cp.wait()
        anchor = bulk(slot // per_grp, (slot % per_grp) * _BULK_ROWS,
                      d_lo=_D_SPLIT if slot < per_chunk else 0)
        for task in side[slot]:
            task(anchor)

    for cp in wo_cp:
        cp.wait()

    qi = lax.broadcasted_iota(jnp.int32, (L, L), 0)
    ki = lax.broadcasted_iota(jnp.int32, (L, L), 1)
    mask = (qi >= seg) | (ki >= seg) | (qi >= ki)
    scale = dh ** -0.5

    def finish(s):
        rows = pl.ds(pl.multiple_of(s * seg, seg), seg)
        sg = _rnd(_rnd(sbuf[...]) * _rnd(_silu(xg[rows, :])))
        obuf[rows, :] = (xb[rows, :].astype(_F32) + sg).astype(_BF16)

    def send(it):
        rows = pl.ds(pl.multiple_of(it * (_UNROLL * seg), _UNROLL * seg), _UNROLL * seg)
        pltpu.make_async_copy(obuf.at[rows], out_hbm.at[rows], osem).start()

    def step(s, mem):
        finish(jnp.maximum(s - 1, 0))
        xr = xn[pl.ds(pl.multiple_of(pre + s * xrows, 8), xrows), :]
        h = jnp.concatenate([xr, mem], axis=0).astype(_BF16)
        wpos = pl.ds(pl.multiple_of(lax.rem(s * xrows, ring_rows), 8), xrows)
        rpos = pl.ds(pl.multiple_of(lax.rem(s * seg + ring_off, ring_rows), 8), seg)
        xresult, presult, probs, heads_out = {}, {}, {}, {}
        acc = [None]

        def stage_a(g):
            ids = [m * heads + g * _G + j for m in range(3) for j in range(_G)]
            t = jnp.dot(h, weights(ids), preferred_element_type=_F32)
            for n, i in enumerate(ids):
                xresult[i] = t[:xrows, n * dh:(n + 1) * dh]
                presult[i] = t[xrows:, n * dh:(n + 1) * dh]

        def stage_w(g):
            for m in range(3):
                for j in range(_G):
                    i = m * heads + g * _G + j
                    ring[i, wpos, :] = xresult.pop(i)

        def rows_of(i):
            return jnp.concatenate([ring[i, rpos, :], presult[i]], axis=0)

        def stage_s(g):
            for j in range(_G):
                hd = g * _G + j
                k = rows_of(heads + hd).astype(_BF16)
                sc = lax.dot_general(rows_of(hd), k, _NT, preferred_element_type=_F32) * scale
                sc = jnp.where(mask, sc, -1000000000.0)
                e = jnp.exp(sc - jnp.max(sc, axis=-1, keepdims=True))
                probs[hd] = (e, 1.0 / jnp.sum(e, axis=-1, keepdims=True))

        def stage_p(g):
            outs = []
            for j in range(_G):
                hd = g * _G + j
                e, inv = probs[hd]
                v = rows_of(2 * heads + hd).astype(_BF16)
                outs.append(jnp.dot(e, v, preferred_element_type=_F32) * inv)
            heads_out[g] = jnp.concatenate(outs, axis=1)

        def stage_o(g):
            n = _G * dh // 2
            wt = jnp.concatenate([wo[j, g * n:(g + 1) * n, :] for j in range(n_col)], axis=1)
            t = jnp.dot(heads_out[g], pltpu.bitcast(wt, _BF16), preferred_element_type=_F32)
            acc[0] = t if acc[0] is None else acc[0] + t

        stages = {"A": stage_a, "W": stage_w, "S": stage_s, "P": stage_p, "O": stage_o}
        for name, g in _schedule(ng):
            stages[name](g)
        sbuf[...] = acc[0][:seg]
        return acc[0][seg:]

    def steps(it, mem):
        for u in range(_UNROLL):
            mem = step(it * _UNROLL + u, mem)

        @pl.when(it > 0)
        def _():
            send(it - 1)

        return mem

    sbuf[...] = jnp.zeros(sbuf.shape, _F32)
    lax.fori_loop(0, n_seg // _UNROLL, steps, mem0_ref[...].astype(_F32))
    finish(n_seg - 1)
    send(n_seg // _UNROLL - 1)
    pltpu.make_async_copy(obuf, obuf, osem).wait()


@functools.partial(jax.jit, static_argnames=("A_seg_len",))
def pallas_recurrent_scan__memory_aug_recurrent_mem_tr__moe_arch_mod__prompt_kernel(
    A_x, A_mem0, A_Wq, A_Wk, A_Wv, A_Wo, A_seg_len,
    B_x, B_w_r, B_w_gate, B_w_up, B_w_down,
):
    del B_x
    B, S, D = A_x.shape
    _, H, Dh = A_Wq.shape
    M = A_mem0.shape[1]
    F = B_w_gate.shape[1]
    seg = int(A_seg_len)
    assert B == 1 and S % seg == 0 and Dh == 128 and D % 128 == 0 and H % _CH == 0
    xrows = seg - M
    pre = S - (S // seg) * xrows
    lcm = int(np.lcm(seg, xrows))
    ring_rows = -(-(pre + xrows) // lcm) * lcm
    n_chunk = 3 * H // _CH
    n_sem = 3 + (n_chunk + 1) + D // 128 + 5

    hbm = pl.BlockSpec(memory_space=pltpu.HBM)
    out = pl.pallas_call(
        functools.partial(_kernel, seg=seg, n_mem=M, heads=H, dh=Dh),
        out_shape=jax.ShapeDtypeStruct((S, D), A_x.dtype),
        in_specs=[hbm] * 10,
        out_specs=hbm,
        scratch_shapes=[
            pltpu.VMEM((S, D), _BF16),
            pltpu.VMEM((S, D), _F32),
            pltpu.VMEM((pre // 2, D), _U32),
            pltpu.VMEM((S, D), _F32),
            pltpu.VMEM((n_chunk, D * _CH // 2, Dh), _U32),
            pltpu.VMEM((3 * H, D // 2, Dh), _U32),
            pltpu.VMEM((D // 128, H * Dh // 2, 128), _U32),
            pltpu.VMEM((3 * H, ring_rows, Dh), _F32),
            pltpu.VMEM((F, D), _BF16),
            pltpu.VMEM((F, D), _BF16),
            pltpu.VMEM((F, D), _BF16),
            pltpu.VMEM((D,), _BF16),
            pltpu.VMEM((M, D), _BF16),
            pltpu.VMEM((seg, D), _F32),
            pltpu.VMEM((S, D), _BF16),
            pltpu.SemaphoreType.DMA((n_sem,)),
            pltpu.SemaphoreType.DMA(()),
        ],
        compiler_params=pltpu.CompilerParams(vmem_limit_bytes=112 * 1024 * 1024),
    )(
        A_x.reshape(S, D), A_mem0.reshape(M, D), A_Wq, A_Wk, A_Wv, A_Wo.reshape(H * Dh, D),
        B_w_r, B_w_gate.T, B_w_up.T, B_w_down,
    )
    return out.reshape(B, S, D)
```

```python
import functools

import jax
import jax.numpy as jnp
import numpy as np
from jax import lax
from jax.experimental import pallas as pl
from jax.experimental.pallas import tpu as pltpu

_F32 = jnp.float32
_BF16 = jnp.bfloat16
_U32 = jnp.uint32
_NT = (((1,), (1,)), ((), ()))

_TOP_C = 8
_G = 4
_CH = 16
_LN_EPS = 1e-05
_LN_BLK = 32
_BULK_ROWS = 128
_UNROLL = 4
_D_SPLIT = 256
_FFN_BLK = 128


def _rnd(v):
    return v.astype(_BF16).astype(_F32)


def _silu(v):
    half = 0.5 * v
    return half * jnp.tanh(half) + half


def _after(v, anchor):
    if anchor is None:
        return v
    keep = (pltpu.bitcast(anchor, jnp.int32) | 1) != 0
    keep = jnp.tile(keep, (v.shape[0] // 8, v.shape[1] // 128))
    return jnp.where(keep, v, jnp.zeros_like(v))


def _schedule(ng):
    toks = []
    for g in range(ng):
        toks.append(("A", g))
        if g >= 1:
            toks.append(("S", g - 1))
        if g >= 2:
            toks.append(("P", g - 2))
        toks.append(("W", g))
    first, second = ng // 4, ng - 3 * ng // 8
    toks += [("O", g) for g in range(first)] + [("S", ng - 1), ("P", ng - 2)]
    toks += [("O", g) for g in range(first, second)] + [("P", ng - 1)]
    toks += [("O", g) for g in range(second, ng)]
    return toks


def _kernel(x_hbm, mem0_hbm, wq_hbm, wk_hbm, wv_hbm, wo_hbm, wr_hbm, wg_hbm, wu_hbm, wd_hbm,
            out_hbm,
            xb, xn, xpre, xg, stg, w, wo, ring, wg, wu, wd, wr_ref, mem0_ref, sbuf, obuf, sems, osem,
            *, seg, n_mem, heads, dh):
    S, D = xb.shape
    n_seg = S // seg
    L = seg + n_mem
    xrows = seg - n_mem
    pre = S - n_seg * xrows
    ring_rows = ring.shape[1]
    ring_off = ring_rows - pre
    n_chunk = 3 * heads // _CH
    n_col = D // 128
    ln_rows = (S - pre) // 4
    ng = heads // _G

    x_parts = [(0, pre), (pre, ln_rows), (pre + ln_rows, S - pre - ln_rows)]
    srcs = [(x_hbm.at[pl.ds(r0, n)], xb.at[pl.ds(r0, n)]) for r0, n in x_parts]
    for c, d0, d1 in [(0, 0, _D_SPLIT), (0, _D_SPLIT, D)] + [(c, 0, D) for c in range(1, n_chunk)]:
        src = (wq_hbm, wk_hbm, wv_hbm)[c // (heads // _CH)].bitcast(_U32)
        h2 = (c % (heads // _CH)) * (_CH // 2)
        srcs.append((src.at[pl.ds(d0, d1 - d0), pl.ds(h2, _CH // 2), :],
                     stg.at[c].reshape(D, _CH // 2, dh).at[pl.ds(d0, d1 - d0)]))
    wo32 = wo_hbm.bitcast(_U32)
    for j in range(n_col):
        srcs.append((wo32.at[:, pl.ds(j * 128, 128)], wo.at[j]))
    srcs += [(wg_hbm, wg), (wu_hbm, wu), (wd_hbm, wd), (wr_hbm, wr_ref), (mem0_hbm, mem0_ref)]
    copies = [pltpu.make_async_copy(a, b, sems.at[i]) for i, (a, b) in enumerate(srcs)]
    x_cp, copies = copies[:len(x_parts)], copies[len(x_parts):]
    w_first, w_cp, copies = copies[0], copies[1:n_chunk + 1], copies[n_chunk + 1:]
    wo_cp, copies = copies[:n_col], copies[n_col:]
    ffn_cp, small_cp = copies[:3], copies[3:]

    for cp in ([x_cp[0], w_first, w_cp[0]] + small_cp + [w_cp[1], x_cp[1], w_cp[2], x_cp[2], w_cp[3], w_cp[4]]
               + ffn_cp + [w_cp[5]] + wo_cp):
        cp.start()

    def layernorm(r0, anchor=None):
        rows = pl.ds(r0, _LN_BLK)
        v = xb[rows, :].astype(_F32)
        v = jnp.concatenate([_after(v[:, :128], anchor), v[:, 128:]], axis=1)
        mean = jnp.mean(v, axis=-1, keepdims=True)
        dev = v - mean
        var = jnp.mean(dev * dev, axis=-1, keepdims=True)
        den = _rnd(jnp.sqrt(_rnd(_rnd(var) + _LN_EPS)))
        y = (_rnd(v - _rnd(mean)) * (1.0 / den)).astype(_BF16)
        if r0 < pre:
            xpre[pl.ds(r0 // 2, _LN_BLK // 2), :] = pltpu.bitcast(y, _U32)
        xn[rows, :] = y.astype(_F32)
        xg[rows, :] = y.astype(_F32)

    def retile(pair, anchor=None, d_lo=0, d_hi=D):
        c, j = divmod(pair, _CH // 2)
        blk = 128
        for d0 in range(d_lo, d_hi, blk):
            u = stg[c, pl.ds(d0 * (_CH // 2) + j, blk, stride=_CH // 2), :]
            lo = pltpu.bitcast(u.astype(jnp.uint16), _U32)
            hi = pltpu.bitcast((u >> 16).astype(jnp.uint16), _U32)
            w[2 * pair, pl.ds(d0 // 2, blk // 2), :] = lo
            w[2 * pair + 1, pl.ds(d0 // 2, blk // 2), :] = hi

    def weights(ids, d_lo=0, d_hi=D):
        rows = pl.ds(d_lo // 2, (d_hi - d_lo) // 2)
        return pltpu.bitcast(jnp.concatenate([w[i, rows, :] for i in ids], axis=1), _BF16)

    def bulk(grp, r0, d_lo=0, d_hi=D):
        ids = [grp * _G + j for j in range(_G)]
        lhs = pltpu.bitcast(xpre[pl.ds(r0 // 2, _BULK_ROWS // 2), d_lo:d_hi], _BF16)
        t = jnp.dot(lhs, weights(ids, d_lo, d_hi), preferred_element_type=_F32)
        rows = pl.ds(ring_off + r0, _BULK_ROWS)
        for j, i in enumerate(ids):
            part = t[:, j * dh:(j + 1) * dh]
            ring[i, rows, :] = part if d_lo == 0 else ring[i, rows, :] + part
        return t[:8, :128]

    sub = lax.broadcasted_iota(jnp.int32, (8, 128), 0)
    lane = lax.broadcasted_iota(jnp.int32, (8, 128), 1)
    logits = {}
    routed = {}

    def router_tile(t, anchor=None):
        wr = jnp.broadcast_to(wr_ref[...].astype(_F32).reshape(1, D), (8, D))
        r = lax.dot_general(wr, xn[pl.ds(t * 128, 128), :].astype(_BF16), _NT,
                            preferred_element_type=_F32)
        b, row = divmod(t, 8)
        logits[b] = r if row == 0 else jnp.where(sub == row, r, logits[b])

    def top_c(anchor=None):
        vals, idxs = [], []
        for b in sorted(logits):
            v = _rnd(logits[b])
            vals.append(jnp.where(v != v, -jnp.inf, v))
            idxs.append((b * 1024 + sub * 128 + lane).astype(_F32))
        sel = []
        r_sel = jnp.zeros((_TOP_C, 128), _F32)
        for k in range(_TOP_C):
            m = functools.reduce(jnp.maximum, vals)
            m = jnp.max(jnp.max(m, axis=1, keepdims=True), axis=0, keepdims=True)
            cand = [jnp.where(v == m, i, float(S)) for v, i in zip(vals, idxs)]
            first = functools.reduce(jnp.minimum, cand)
            first = jnp.min(jnp.min(first, axis=1, keepdims=True), axis=0, keepdims=True)
            vals = [jnp.where(i == first, -jnp.inf, v) for v, i in zip(vals, idxs)]
            idxs = [jnp.where(i == first, float(S), i) for i in idxs]
            r_sel = jnp.where(sub == k, m, r_sel)
            sel.append(jnp.clip(first[0, 0].astype(jnp.int32), 0, S - 1))
        routed["sel"] = sel
        routed["r"] = r_sel[:, 0:1]
        routed["x"] = jnp.concatenate([xn[pl.ds(tok, 1), :] for tok in sel], axis=0)

    n_ffn = wg.shape[0]
    ffn_blocks = [(f0, min(_FFN_BLK, n_ffn - f0)) for f0 in range(0, n_ffn, _FFN_BLK)]

    def expert_hidden(n, anchor=None):
        f0, fn = ffn_blocks[n]
        hg = lax.dot_general(routed["x"], wg[pl.ds(f0, fn), :], _NT, preferred_element_type=_F32)
        hu = lax.dot_general(routed["x"], wu[pl.ds(f0, fn), :], _NT, preferred_element_type=_F32)
        routed[n] = _rnd(_silu(_rnd(hg))) * _rnd(hu)

    def expert_down(n, anchor=None):
        f0, fn = ffn_blocks[n]
        t = jnp.dot(routed.pop(n), wd[pl.ds(f0, fn), :], preferred_element_type=_F32)
        routed["y"] = t if n == 0 else routed["y"] + t

    def expert_scatter(anchor=None):
        y = _rnd(_rnd(routed["y"]) * _rnd(jax.nn.sigmoid(routed["r"])))
        rows = _rnd(routed["x"] + y)
        for k, tok in enumerate(routed["sel"]):
            xg[pl.ds(tok, 1), :] = rows[k:k + 1, :]

    per_grp = pre // _BULK_ROWS
    per_chunk = per_grp * (_CH // _G)
    n_slot = per_chunk * n_chunk
    waits = {per_chunk - per_grp: [w_cp[1], x_cp[1]] + small_cp,
             2 * per_chunk - per_grp: [w_cp[2], x_cp[2]],
             3 * per_chunk - per_grp: [w_cp[3], w_cp[4]],
             4 * per_chunk: ffn_cp,
             5 * per_chunk - per_grp: [w_cp[5]]}
    side = [[] for _ in range(n_slot)]

    def spread(tasks, first, last):
        for n, task in enumerate(tasks):
            side[first + n * (last - first + 1) // len(tasks)].append(task)

    def ln_tasks(part):
        r0, n = x_parts[part]
        return [functools.partial(layernorm, r) for r in range(r0, r0 + n, _LN_BLK)]

    def router_tasks(part):
        r0, n = x_parts[part]
        return [functools.partial(router_tile, t) for t in range(r0 // 128, (r0 + n) // 128)]

    for grp in range(1, n_slot // per_grp):
        for j in range(_G // 2):
            side[(grp - 1) * per_grp + j].append(functools.partial(
                retile, grp * (_G // 2) + j, d_lo=_D_SPLIT if grp < _CH // _G else 0))
    b1, b2, b3, b4, _ = sorted(waits)
    late_ln = ln_tasks(2)
    spread(ln_tasks(1), b1 + 1, b2 - 3)
    spread(router_tasks(0), b1 + 1, b2 - 3)
    spread(late_ln[:len(late_ln) // 2], b2 + 1, b3 - 3)
    spread(router_tasks(1), b2 + 1, b3 - 3)
    spread(late_ln[len(late_ln) // 2:], b3 + 1, b3 + 10)
    spread(router_tasks(2), b3 + 4, b4 - 7)
    side[b4 - 7].append(top_c)
    spread([functools.partial(fn, n) for n in range(len(ffn_blocks))
            for fn in (expert_hidden, expert_down)] + [expert_scatter], b4, n_slot - 3)

    x_cp[0].wait()
    for task in ln_tasks(0):
        task()
    w_first.wait()
    for pair in range(_CH // 2):
        retile(pair, d_hi=_D_SPLIT)
    for slot in range(per_chunk):
        bulk(slot // per_grp, (slot % per_grp) * _BULK_ROWS, d_hi=_D_SPLIT)
    w_cp[0].wait()
    for j in range(_G // 2):
        retile(j, d_lo=_D_SPLIT)
    for slot in range(n_slot):
        for cp in waits.get(slot, []):
            cp.wait()
        anchor = bulk(slot // per_grp, (slot % per_grp) * _BULK_ROWS,
                      d_lo=_D_SPLIT if slot < per_chunk else 0)
        for task in side[slot]:
            task(anchor)

    for cp in wo_cp:
        cp.wait()

    qi = lax.broadcasted_iota(jnp.int32, (L, L), 0)
    ki = lax.broadcasted_iota(jnp.int32, (L, L), 1)
    mask = (qi >= seg) | (ki >= seg) | (qi >= ki)
    scale = dh ** -0.5

    def finish(s):
        rows = pl.ds(pl.multiple_of(s * seg, seg), seg)
        sg = _rnd(_rnd(sbuf[...]) * _rnd(_silu(xg[rows, :])))
        obuf[rows, :] = (xb[rows, :].astype(_F32) + sg).astype(_BF16)

    def send(r0, n):
        pltpu.make_async_copy(obuf.at[pl.ds(r0, n)], out_hbm.at[pl.ds(r0, n)], osem).start()

    def step(s, mem):
        finish(jnp.maximum(s - 1, 0))
        xr = xn[pl.ds(pl.multiple_of(pre + s * xrows, 8), xrows), :]
        h = jnp.concatenate([xr, mem], axis=0).astype(_BF16)
        wpos = pl.ds(pl.multiple_of(lax.rem(s * xrows, ring_rows), 8), xrows)
        rpos = pl.ds(pl.multiple_of(lax.rem(s * seg + ring_off, ring_rows), 8), seg)
        xresult, presult, probs, heads_out = {}, {}, {}, {}
        acc = [None]

        def stage_a(g):
            ids = [m * heads + g * _G + j for m in range(3) for j in range(_G)]
            t = jnp.dot(h, weights(ids), preferred_element_type=_F32)
            for n, i in enumerate(ids):
                xresult[i] = t[:xrows, n * dh:(n + 1) * dh]
                presult[i] = t[xrows:, n * dh:(n + 1) * dh]

        def stage_w(g):
            for m in range(3):
                for j in range(_G):
                    i = m * heads + g * _G + j
                    ring[i, wpos, :] = xresult.pop(i)

        def rows_of(i):
            return jnp.concatenate([ring[i, rpos, :], presult[i]], axis=0)

        def stage_s(g):
            for j in range(_G):
                hd = g * _G + j
                k = rows_of(heads + hd).astype(_BF16)
                sc = lax.dot_general(rows_of(hd), k, _NT, preferred_element_type=_F32) * scale
                sc = jnp.where(mask, sc, -1000000000.0)
                e = jnp.exp(sc - jnp.max(sc, axis=-1, keepdims=True))
                probs[hd] = (e, 1.0 / jnp.sum(e, axis=-1, keepdims=True))

        def stage_p(g):
            outs = []
            for j in range(_G):
                hd = g * _G + j
                e, inv = probs[hd]
                v = rows_of(2 * heads + hd).astype(_BF16)
                outs.append(jnp.dot(e, v, preferred_element_type=_F32) * inv)
            heads_out[g] = jnp.concatenate(outs, axis=1)

        def stage_o(g):
            n = _G * dh // 2
            wt = jnp.concatenate([wo[j, g * n:(g + 1) * n, :] for j in range(n_col)], axis=1)
            t = jnp.dot(heads_out[g], pltpu.bitcast(wt, _BF16), preferred_element_type=_F32)
            acc[0] = t if acc[0] is None else acc[0] + t

        stages = {"A": stage_a, "W": stage_w, "S": stage_s, "P": stage_p, "O": stage_o}
        for name, g in _schedule(ng):
            stages[name](g)
        sbuf[...] = acc[0][:seg]
        return acc[0][seg:]

    def steps(it, mem):
        for u in range(_UNROLL):
            mem = step(it * _UNROLL + u, mem)

        @pl.when(it > 0)
        def _():
            send(pl.multiple_of((it - 1) * (_UNROLL * seg), _UNROLL * seg), _UNROLL * seg)

        return mem

    sbuf[...] = jnp.zeros(sbuf.shape, _F32)
    lax.fori_loop(0, n_seg // _UNROLL, steps, mem0_ref[...].astype(_F32))
    send(S - _UNROLL * seg, (_UNROLL - 1) * seg)
    finish(n_seg - 1)
    send(S - seg, seg)
    pltpu.make_async_copy(obuf, obuf, osem).wait()


@functools.partial(jax.jit, static_argnames=("A_seg_len",))
def pallas_recurrent_scan__memory_aug_recurrent_mem_tr__moe_arch_mod__prompt_kernel(
    A_x, A_mem0, A_Wq, A_Wk, A_Wv, A_Wo, A_seg_len,
    B_x, B_w_r, B_w_gate, B_w_up, B_w_down,
):
    del B_x
    B, S, D = A_x.shape
    _, H, Dh = A_Wq.shape
    M = A_mem0.shape[1]
    F = B_w_gate.shape[1]
    seg = int(A_seg_len)
    assert B == 1 and S % seg == 0 and Dh == 128 and D % 128 == 0 and H % _CH == 0
    xrows = seg - M
    pre = S - (S // seg) * xrows
    lcm = int(np.lcm(seg, xrows))
    ring_rows = -(-(pre + xrows) // lcm) * lcm
    n_chunk = 3 * H // _CH
    n_sem = 3 + (n_chunk + 1) + D // 128 + 5

    hbm = pl.BlockSpec(memory_space=pltpu.HBM)
    out = pl.pallas_call(
        functools.partial(_kernel, seg=seg, n_mem=M, heads=H, dh=Dh),
        out_shape=jax.ShapeDtypeStruct((S, D), A_x.dtype),
        in_specs=[hbm] * 10,
        out_specs=hbm,
        scratch_shapes=[
            pltpu.VMEM((S, D), _BF16),
            pltpu.VMEM((S, D), _F32),
            pltpu.VMEM((pre // 2, D), _U32),
            pltpu.VMEM((S, D), _F32),
            pltpu.VMEM((n_chunk, D * _CH // 2, Dh), _U32),
            pltpu.VMEM((3 * H, D // 2, Dh), _U32),
            pltpu.VMEM((D // 128, H * Dh // 2, 128), _U32),
            pltpu.VMEM((3 * H, ring_rows, Dh), _F32),
            pltpu.VMEM((F, D), _BF16),
            pltpu.VMEM((F, D), _BF16),
            pltpu.VMEM((F, D), _BF16),
            pltpu.VMEM((D,), _BF16),
            pltpu.VMEM((M, D), _BF16),
            pltpu.VMEM((seg, D), _F32),
            pltpu.VMEM((S, D), _BF16),
            pltpu.SemaphoreType.DMA((n_sem,)),
            pltpu.SemaphoreType.DMA(()),
        ],
        compiler_params=pltpu.CompilerParams(vmem_limit_bytes=112 * 1024 * 1024),
    )(
        A_x.reshape(S, D), A_mem0.reshape(M, D), A_Wq, A_Wk, A_Wv, A_Wo.reshape(H * Dh, D),
        B_w_r, B_w_gate.T, B_w_up.T, B_w_down,
    )
    return out.reshape(B, S, D)
```

```python
import functools

import jax
import jax.numpy as jnp
import numpy as np
from jax import lax
from jax.experimental import pallas as pl
from jax.experimental.pallas import tpu as pltpu

_F32 = jnp.float32
_BF16 = jnp.bfloat16
_U32 = jnp.uint32
_NT = (((1,), (1,)), ((), ()))

_TOP_C = 8
_G = 4
_CH = 16
_LN_EPS = 1e-05
_LN_BLK = 32
_BULK_ROWS = 128
_UNROLL = 4
_D_SPLIT = 256
_FFN_BLK = 128


def _rnd(v):
    return v.astype(_BF16).astype(_F32)


def _silu(v):
    half = 0.5 * v
    return half * jnp.tanh(half) + half


def _after(v, anchor):
    if anchor is None:
        return v
    keep = (pltpu.bitcast(anchor, jnp.int32) | 1) != 0
    keep = jnp.tile(keep, (v.shape[0] // 8, v.shape[1] // 128))
    return jnp.where(keep, v, jnp.zeros_like(v))


def _schedule(ng):
    toks = []
    for g in range(ng):
        toks.append(("A", g))
        if g >= 1:
            toks.append(("S", g - 1))
        if g >= 2:
            toks.append(("P", g - 2))
        toks.append(("W", g))
    first, second = ng // 4, ng - 3 * ng // 8
    toks += [("O", g) for g in range(first)] + [("S", ng - 1), ("P", ng - 2)]
    toks += [("O", g) for g in range(first, second)] + [("P", ng - 1)]
    toks += [("O", g) for g in range(second, ng)]
    return toks


def _kernel(x_hbm, mem0_hbm, wq_hbm, wk_hbm, wv_hbm, wo_hbm, wr_hbm, wg_hbm, wu_hbm, wd_hbm,
            out_hbm,
            xb, xn, xpre, xg, stg, w, wo, ring, wg, wu, wd, wr_ref, mem0_ref, sbuf, obuf, sems, osem,
            *, seg, n_mem, heads, dh):
    S, D = xb.shape
    n_seg = S // seg
    L = seg + n_mem
    xrows = seg - n_mem
    pre = S - n_seg * xrows
    ring_rows = ring.shape[1]
    ring_off = ring_rows - pre
    n_chunk = 3 * heads // _CH
    n_col = D // 128
    ln_rows = (S - pre) // 4
    ng = heads // _G

    x_parts = [(0, pre), (pre, ln_rows), (pre + ln_rows, S - pre - ln_rows)]
    srcs = [(x_hbm.at[pl.ds(r0, n)], xb.at[pl.ds(r0, n)]) for r0, n in x_parts]
    for c, d0, d1 in [(0, 0, _D_SPLIT), (0, _D_SPLIT, D)] + [(c, 0, D) for c in range(1, n_chunk)]:
        src = (wq_hbm, wk_hbm, wv_hbm)[c // (heads // _CH)].bitcast(_U32)
        h2 = (c % (heads // _CH)) * (_CH // 2)
        srcs.append((src.at[pl.ds(d0, d1 - d0), pl.ds(h2, _CH // 2), :],
                     stg.at[c].reshape(D, _CH // 2, dh).at[pl.ds(d0, d1 - d0)]))
    wo32 = wo_hbm.bitcast(_U32)
    for j in range(n_col):
        srcs.append((wo32.at[:, pl.ds(j * 128, 128)], wo.at[j]))
    srcs += [(wg_hbm, wg), (wu_hbm, wu), (wd_hbm, wd), (wr_hbm, wr_ref), (mem0_hbm, mem0_ref)]
    copies = [pltpu.make_async_copy(a, b, sems.at[i]) for i, (a, b) in enumerate(srcs)]
    x_cp, copies = copies[:len(x_parts)], copies[len(x_parts):]
    w_first, w_cp, copies = copies[0], copies[1:n_chunk + 1], copies[n_chunk + 1:]
    wo_cp, copies = copies[:n_col], copies[n_col:]
    ffn_cp, small_cp = copies[:3], copies[3:]

    for cp in ([x_cp[0], w_first, w_cp[0]] + small_cp + [w_cp[1], x_cp[1], w_cp[2], x_cp[2], w_cp[3], w_cp[4]]
               + ffn_cp + [w_cp[5]] + wo_cp):
        cp.start()

    def layernorm(r0, anchor=None):
        rows = pl.ds(r0, _LN_BLK)
        v = xb[rows, :].astype(_F32)
        v = jnp.concatenate([_after(v[:, :128], anchor), v[:, 128:]], axis=1)
        mean = jnp.mean(v, axis=-1, keepdims=True)
        dev = v - mean
        var = jnp.mean(dev * dev, axis=-1, keepdims=True)
        den = _rnd(jnp.sqrt(_rnd(_rnd(var) + _LN_EPS)))
        y = (_rnd(v - _rnd(mean)) * (1.0 / den)).astype(_BF16)
        if r0 < pre:
            xpre[pl.ds(r0 // 2, _LN_BLK // 2), :] = pltpu.bitcast(y, _U32)
        xn[rows, :] = y.astype(_F32)
        xg[rows, :] = y.astype(_F32)

    def retile(pair, anchor=None, d_lo=0, d_hi=D):
        c, j = divmod(pair, _CH // 2)
        blk = 128
        for d0 in range(d_lo, d_hi, blk):
            u = stg[c, pl.ds(d0 * (_CH // 2) + j, blk, stride=_CH // 2), :]
            lo = pltpu.bitcast(u.astype(jnp.uint16), _U32)
            hi = pltpu.bitcast((u >> 16).astype(jnp.uint16), _U32)
            w[2 * pair, pl.ds(d0 // 2, blk // 2), :] = lo
            w[2 * pair + 1, pl.ds(d0 // 2, blk // 2), :] = hi

    def weights(ids, d_lo=0, d_hi=D):
        rows = pl.ds(d_lo // 2, (d_hi - d_lo) // 2)
        return pltpu.bitcast(jnp.concatenate([w[i, rows, :] for i in ids], axis=1), _BF16)

    def bulk(grp, r0, d_lo=0, d_hi=D):
        ids = [grp * _G + j for j in range(_G)]
        lhs = pltpu.bitcast(xpre[pl.ds(r0 // 2, _BULK_ROWS // 2), d_lo:d_hi], _BF16)
        t = jnp.dot(lhs, weights(ids, d_lo, d_hi), preferred_element_type=_F32)
        rows = pl.ds(ring_off + r0, _BULK_ROWS)
        for j, i in enumerate(ids):
            part = t[:, j * dh:(j + 1) * dh]
            ring[i, rows, :] = part if d_lo == 0 else ring[i, rows, :] + part
        return t[:8, :128]

    sub = lax.broadcasted_iota(jnp.int32, (8, 128), 0)
    lane = lax.broadcasted_iota(jnp.int32, (8, 128), 1)
    logits = {}
    routed = {}

    def router_tile(t, anchor=None):
        wr = jnp.broadcast_to(wr_ref[...].astype(_F32).reshape(1, D), (8, D))
        r = lax.dot_general(wr, xn[pl.ds(t * 128, 128), :].astype(_BF16), _NT,
                            preferred_element_type=_F32)
        b, row = divmod(t, 8)
        logits[b] = r if row == 0 else jnp.where(sub == row, r, logits[b])

    def top_c(anchor=None):
        vals, idxs = [], []
        for b in sorted(logits):
            v = _rnd(logits[b])
            vals.append(jnp.where(v != v, -jnp.inf, v))
            idxs.append((b * 1024 + sub * 128 + lane).astype(_F32))
        sel = []
        r_sel = jnp.zeros((_TOP_C, 128), _F32)
        for k in range(_TOP_C):
            m = functools.reduce(jnp.maximum, vals)
            m = jnp.max(jnp.max(m, axis=1, keepdims=True), axis=0, keepdims=True)
            cand = [jnp.where(v == m, i, float(S)) for v, i in zip(vals, idxs)]
            first = functools.reduce(jnp.minimum, cand)
            first = jnp.min(jnp.min(first, axis=1, keepdims=True), axis=0, keepdims=True)
            vals = [jnp.where(i == first, -jnp.inf, v) for v, i in zip(vals, idxs)]
            idxs = [jnp.where(i == first, float(S), i) for i in idxs]
            r_sel = jnp.where(sub == k, m, r_sel)
            sel.append(jnp.clip(first[0, 0].astype(jnp.int32), 0, S - 1))
        routed["sel"] = sel
        routed["r"] = r_sel[:, 0:1]
        routed["x"] = jnp.concatenate([xn[pl.ds(tok, 1), :] for tok in sel], axis=0)

    n_ffn = wg.shape[0]
    ffn_blocks = [(f0, min(_FFN_BLK, n_ffn - f0)) for f0 in range(0, n_ffn, _FFN_BLK)]

    def expert_hidden(n, anchor=None):
        f0, fn = ffn_blocks[n]
        hg = lax.dot_general(routed["x"], wg[pl.ds(f0, fn), :], _NT, preferred_element_type=_F32)
        hu = lax.dot_general(routed["x"], wu[pl.ds(f0, fn), :], _NT, preferred_element_type=_F32)
        routed[n] = _rnd(_silu(_rnd(hg))) * _rnd(hu)

    def expert_down(n, anchor=None):
        f0, fn = ffn_blocks[n]
        t = jnp.dot(routed.pop(n), wd[pl.ds(f0, fn), :], preferred_element_type=_F32)
        routed["y"] = t if n == 0 else routed["y"] + t

    def expert_scatter(anchor=None):
        y = _rnd(_rnd(routed["y"]) * _rnd(jax.nn.sigmoid(routed["r"])))
        rows = _rnd(routed["x"] + y)
        for k, tok in enumerate(routed["sel"]):
            xg[pl.ds(tok, 1), :] = rows[k:k + 1, :]

    per_grp = pre // _BULK_ROWS
    per_chunk = per_grp * (_CH // _G)
    n_slot = per_chunk * n_chunk
    waits = {per_chunk - per_grp: [w_cp[1], x_cp[1]] + small_cp,
             2 * per_chunk - per_grp: [w_cp[2], x_cp[2]],
             3 * per_chunk - per_grp: [w_cp[3], w_cp[4]],
             4 * per_chunk: ffn_cp,
             5 * per_chunk - per_grp: [w_cp[5]]}
    side = [[] for _ in range(n_slot)]

    def spread(tasks, first, last):
        for n, task in enumerate(tasks):
            side[first + n * (last - first + 1) // len(tasks)].append(task)

    def ln_tasks(part):
        r0, n = x_parts[part]
        return [functools.partial(layernorm, r) for r in range(r0, r0 + n, _LN_BLK)]

    def router_tasks(part):
        r0, n = x_parts[part]
        return [functools.partial(router_tile, t) for t in range(r0 // 128, (r0 + n) // 128)]

    for grp in range(1, n_slot // per_grp):
        for j in range(_G // 2):
            side[(grp - 1) * per_grp + j].append(functools.partial(
                retile, grp * (_G // 2) + j, d_lo=_D_SPLIT if grp < _CH // _G else 0))
    b1, b2, b3, b4, _ = sorted(waits)
    late_ln = ln_tasks(2)
    spread(ln_tasks(1), b1 + 1, b2 - 3)
    spread(router_tasks(0), b1 + 1, b2 - 3)
    spread(late_ln[:len(late_ln) // 2], b2 + 1, b3 - 3)
    spread(router_tasks(1), b2 + 1, b3 - 3)
    spread(late_ln[len(late_ln) // 2:], b3 + 1, b3 + 10)
    spread(router_tasks(2), b3 + 4, b4 - 7)
    side[b4 - 7].append(top_c)
    spread([functools.partial(fn, n) for n in range(len(ffn_blocks))
            for fn in (expert_hidden, expert_down)] + [expert_scatter], b4, n_slot - 3)

    x_cp[0].wait()
    for task in ln_tasks(0):
        task()
    w_first.wait()
    for pair in range(_CH // 2):
        retile(pair, d_hi=_D_SPLIT)
    for slot in range(per_chunk):
        j = slot - (per_chunk - per_grp)
        if j == 0:
            w_cp[0].wait()
        anchor = bulk(slot // per_grp, (slot % per_grp) * _BULK_ROWS, d_hi=_D_SPLIT)
        if 0 <= j < _G // 2:
            retile(j, anchor, d_lo=_D_SPLIT)
    for slot in range(n_slot):
        for cp in waits.get(slot, []):
            cp.wait()
        anchor = bulk(slot // per_grp, (slot % per_grp) * _BULK_ROWS,
                      d_lo=_D_SPLIT if slot < per_chunk else 0)
        for task in side[slot]:
            task(anchor)

    for cp in wo_cp:
        cp.wait()

    qi = lax.broadcasted_iota(jnp.int32, (L, L), 0)
    ki = lax.broadcasted_iota(jnp.int32, (L, L), 1)
    mask = (qi >= seg) | (ki >= seg) | (qi >= ki)
    scale = dh ** -0.5

    def finish(s):
        rows = pl.ds(pl.multiple_of(s * seg, seg), seg)
        sg = _rnd(_rnd(sbuf[...]) * _rnd(_silu(xg[rows, :])))
        obuf[rows, :] = (xb[rows, :].astype(_F32) + sg).astype(_BF16)

    def send(r0, n):
        pltpu.make_async_copy(obuf.at[pl.ds(r0, n)], out_hbm.at[pl.ds(r0, n)], osem).start()

    def step(s, mem):
        finish(jnp.maximum(s - 1, 0))
        xr = xn[pl.ds(pl.multiple_of(pre + s * xrows, 8), xrows), :]
        h = jnp.concatenate([xr, mem], axis=0).astype(_BF16)
        wpos = pl.ds(pl.multiple_of(lax.rem(s * xrows, ring_rows), 8), xrows)
        rpos = pl.ds(pl.multiple_of(lax.rem(s * seg + ring_off, ring_rows), 8), seg)
        xresult, presult, probs, heads_out = {}, {}, {}, {}
        acc = [None]

        def stage_a(g):
            ids = [m * heads + g * _G + j for m in range(3) for j in range(_G)]
            t = jnp.dot(h, weights(ids), preferred_element_type=_F32)
            for n, i in enumerate(ids):
                xresult[i] = t[:xrows, n * dh:(n + 1) * dh]
                presult[i] = t[xrows:, n * dh:(n + 1) * dh]

        def stage_w(g):
            for m in range(3):
                for j in range(_G):
                    i = m * heads + g * _G + j
                    ring[i, wpos, :] = xresult.pop(i)

        def rows_of(i):
            return jnp.concatenate([ring[i, rpos, :], presult[i]], axis=0)

        def stage_s(g):
            for j in range(_G):
                hd = g * _G + j
                k = rows_of(heads + hd).astype(_BF16)
                sc = lax.dot_general(rows_of(hd), k, _NT, preferred_element_type=_F32) * scale
                sc = jnp.where(mask, sc, -1000000000.0)
                e = jnp.exp(sc - jnp.max(sc, axis=-1, keepdims=True))
                probs[hd] = (e, 1.0 / jnp.sum(e, axis=-1, keepdims=True))

        def stage_p(g):
            outs = []
            for j in range(_G):
                hd = g * _G + j
                e, inv = probs[hd]
                v = rows_of(2 * heads + hd).astype(_BF16)
                outs.append(jnp.dot(e, v, preferred_element_type=_F32) * inv)
            heads_out[g] = jnp.concatenate(outs, axis=1)

        def stage_o(g):
            n = _G * dh // 2
            wt = jnp.concatenate([wo[j, g * n:(g + 1) * n, :] for j in range(n_col)], axis=1)
            t = jnp.dot(heads_out[g], pltpu.bitcast(wt, _BF16), preferred_element_type=_F32)
            acc[0] = t if acc[0] is None else acc[0] + t

        stages = {"A": stage_a, "W": stage_w, "S": stage_s, "P": stage_p, "O": stage_o}
        for name, g in _schedule(ng):
            stages[name](g)
        sbuf[...] = acc[0][:seg]
        return acc[0][seg:]

    def steps(it, mem):
        for u in range(_UNROLL):
            mem = step(it * _UNROLL + u, mem)

        @pl.when(it > 0)
        def _():
            send(pl.multiple_of((it - 1) * (_UNROLL * seg), _UNROLL * seg), _UNROLL * seg)

        return mem

    sbuf[...] = jnp.zeros(sbuf.shape, _F32)
    lax.fori_loop(0, n_seg // _UNROLL, steps, mem0_ref[...].astype(_F32))
    send(S - _UNROLL * seg, (_UNROLL - 1) * seg)
    finish(n_seg - 1)
    send(S - seg, seg)
    pltpu.make_async_copy(obuf, obuf, osem).wait()


@functools.partial(jax.jit, static_argnames=("A_seg_len",))
def pallas_recurrent_scan__memory_aug_recurrent_mem_tr__moe_arch_mod__prompt_kernel(
    A_x, A_mem0, A_Wq, A_Wk, A_Wv, A_Wo, A_seg_len,
    B_x, B_w_r, B_w_gate, B_w_up, B_w_down,
):
    del B_x
    B, S, D = A_x.shape
    _, H, Dh = A_Wq.shape
    M = A_mem0.shape[1]
    F = B_w_gate.shape[1]
    seg = int(A_seg_len)
    assert B == 1 and S % seg == 0 and Dh == 128 and D % 128 == 0 and H % _CH == 0
    xrows = seg - M
    pre = S - (S // seg) * xrows
    lcm = int(np.lcm(seg, xrows))
    ring_rows = -(-(pre + xrows) // lcm) * lcm
    n_chunk = 3 * H // _CH
    n_sem = 3 + (n_chunk + 1) + D // 128 + 5

    hbm = pl.BlockSpec(memory_space=pltpu.HBM)
    out = pl.pallas_call(
        functools.partial(_kernel, seg=seg, n_mem=M, heads=H, dh=Dh),
        out_shape=jax.ShapeDtypeStruct((S, D), A_x.dtype),
        in_specs=[hbm] * 10,
        out_specs=hbm,
        scratch_shapes=[
            pltpu.VMEM((S, D), _BF16),
            pltpu.VMEM((S, D), _F32),
            pltpu.VMEM((pre // 2, D), _U32),
            pltpu.VMEM((S, D), _F32),
            pltpu.VMEM((n_chunk, D * _CH // 2, Dh), _U32),
            pltpu.VMEM((3 * H, D // 2, Dh), _U32),
            pltpu.VMEM((D // 128, H * Dh // 2, 128), _U32),
            pltpu.VMEM((3 * H, ring_rows, Dh), _F32),
            pltpu.VMEM((F, D), _BF16),
            pltpu.VMEM((F, D), _BF16),
            pltpu.VMEM((F, D), _BF16),
            pltpu.VMEM((D,), _BF16),
            pltpu.VMEM((M, D), _BF16),
            pltpu.VMEM((seg, D), _F32),
            pltpu.VMEM((S, D), _BF16),
            pltpu.SemaphoreType.DMA((n_sem,)),
            pltpu.SemaphoreType.DMA(()),
        ],
        compiler_params=pltpu.CompilerParams(vmem_limit_bytes=112 * 1024 * 1024),
    )(
        A_x.reshape(S, D), A_mem0.reshape(M, D), A_Wq, A_Wk, A_Wv, A_Wo.reshape(H * Dh, D),
        B_w_r, B_w_gate.T, B_w_up.T, B_w_down,
    )
    return out.reshape(B, S, D)
```

```python
import functools

import jax
import jax.numpy as jnp
import numpy as np
from jax import lax
from jax.experimental import pallas as pl
from jax.experimental.pallas import tpu as pltpu

_F32 = jnp.float32
_BF16 = jnp.bfloat16
_U32 = jnp.uint32
_NT = (((1,), (1,)), ((), ()))

_TOP_C = 8
_G = 4
_CH = 16
_LN_EPS = 1e-05
_LN_BLK = 32
_BULK_ROWS = 128
_UNROLL = 4
_D_SPLIT = 256
_FFN_BLK = 128


def _rnd(v):
    return v.astype(_BF16).astype(_F32)


def _silu(v):
    half = 0.5 * v
    return half * jnp.tanh(half) + half


def _after(v, anchor):
    if anchor is None:
        return v
    keep = (pltpu.bitcast(anchor, jnp.int32) | 1) != 0
    keep = jnp.tile(keep, (v.shape[0] // 8, v.shape[1] // 128))
    return jnp.where(keep, v, jnp.zeros_like(v))


def _schedule(ng):
    toks = []
    for g in range(ng):
        toks.append(("A", g))
        if g >= 1:
            toks.append(("S", g - 1))
        if g >= 2:
            toks.append(("P", g - 2))
        toks.append(("W", g))
    first, second = ng // 4, ng - 3 * ng // 8
    toks += [("O", g) for g in range(first)] + [("S", ng - 1), ("P", ng - 2)]
    toks += [("O", g) for g in range(first, second)] + [("P", ng - 1)]
    toks += [("O", g) for g in range(second, ng)]
    return toks


def _kernel(x_hbm, mem0_hbm, wq_hbm, wk_hbm, wv_hbm, wo_hbm, wr_hbm, wg_hbm, wu_hbm, wd_hbm,
            out_hbm,
            stg, wg, wu, wd, wr_ref, mem0_ref, xpre, w, wo, ring, xb, obuf, xg, xn, sbuf, sems, osem,
            *, seg, n_mem, heads, dh):
    S, D = xb.shape
    n_seg = S // seg
    L = seg + n_mem
    xrows = seg - n_mem
    pre = S - n_seg * xrows
    ring_rows = ring.shape[1]
    ring_off = ring_rows - pre
    n_chunk = 3 * heads // _CH
    n_col = D // 128
    ln_rows = (S - pre) // 4
    ng = heads // _G

    x_parts = [(0, pre), (pre, ln_rows), (pre + ln_rows, S - pre - ln_rows)]
    srcs = [(x_hbm.at[pl.ds(r0, n)], xb.at[pl.ds(r0, n)]) for r0, n in x_parts]
    for c, d0, d1 in [(0, 0, _D_SPLIT), (0, _D_SPLIT, D)] + [(c, 0, D) for c in range(1, n_chunk)]:
        src = (wq_hbm, wk_hbm, wv_hbm)[c // (heads // _CH)].bitcast(_U32)
        h2 = (c % (heads // _CH)) * (_CH // 2)
        srcs.append((src.at[pl.ds(d0, d1 - d0), pl.ds(h2, _CH // 2), :],
                     stg.at[c].reshape(D, _CH // 2, dh).at[pl.ds(d0, d1 - d0)]))
    wo32 = wo_hbm.bitcast(_U32)
    for j in range(n_col):
        srcs.append((wo32.at[:, pl.ds(j * 128, 128)], wo.at[j]))
    srcs += [(wg_hbm, wg), (wu_hbm, wu), (wd_hbm, wd), (wr_hbm, wr_ref), (mem0_hbm, mem0_ref)]
    copies = [pltpu.make_async_copy(a, b, sems.at[i]) for i, (a, b) in enumerate(srcs)]
    x_cp, copies = copies[:len(x_parts)], copies[len(x_parts):]
    w_first, w_cp, copies = copies[0], copies[1:n_chunk + 1], copies[n_chunk + 1:]
    wo_cp, copies = copies[:n_col], copies[n_col:]
    ffn_cp, small_cp = copies[:3], copies[3:]

    for cp in ([x_cp[0], w_first, w_cp[0]] + small_cp + [w_cp[1], x_cp[1], w_cp[2], x_cp[2], w_cp[3], w_cp[4]]
               + ffn_cp + [w_cp[5]] + wo_cp):
        cp.start()

    def layernorm(r0, anchor=None):
        rows = pl.ds(r0, _LN_BLK)
        v = xb[rows, :].astype(_F32)
        v = jnp.concatenate([_after(v[:, :128], anchor), v[:, 128:]], axis=1)
        mean = jnp.mean(v, axis=-1, keepdims=True)
        dev = v - mean
        var = jnp.mean(dev * dev, axis=-1, keepdims=True)
        den = _rnd(jnp.sqrt(_rnd(_rnd(var) + _LN_EPS)))
        y = (_rnd(v - _rnd(mean)) * (1.0 / den)).astype(_BF16)
        if r0 < pre:
            xpre[pl.ds(r0 // 2, _LN_BLK // 2), :] = pltpu.bitcast(y, _U32)
        xn[rows, :] = y.astype(_F32)
        xg[rows, :] = y.astype(_F32)

    def retile(pair, anchor=None, d_lo=0, d_hi=D):
        c, j = divmod(pair, _CH // 2)
        blk = 128
        for d0 in range(d_lo, d_hi, blk):
            u = stg[c, pl.ds(d0 * (_CH // 2) + j, blk, stride=_CH // 2), :]
            lo = pltpu.bitcast(u.astype(jnp.uint16), _U32)
            hi = pltpu.bitcast((u >> 16).astype(jnp.uint16), _U32)
            w[2 * pair, pl.ds(d0 // 2, blk // 2), :] = lo
            w[2 * pair + 1, pl.ds(d0 // 2, blk // 2), :] = hi

    def weights(ids, d_lo=0, d_hi=D):
        rows = pl.ds(d_lo // 2, (d_hi - d_lo) // 2)
        return pltpu.bitcast(jnp.concatenate([w[i, rows, :] for i in ids], axis=1), _BF16)

    def bulk(grp, r0, d_lo=0, d_hi=D):
        ids = [grp * _G + j for j in range(_G)]
        lhs = pltpu.bitcast(xpre[pl.ds(r0 // 2, _BULK_ROWS // 2), d_lo:d_hi], _BF16)
        t = jnp.dot(lhs, weights(ids, d_lo, d_hi), preferred_element_type=_F32)
        rows = pl.ds(ring_off + r0, _BULK_ROWS)
        for j, i in enumerate(ids):
            part = t[:, j * dh:(j + 1) * dh]
            ring[i, rows, :] = part if d_lo == 0 else ring[i, rows, :] + part
        return t[:8, :128]

    sub = lax.broadcasted_iota(jnp.int32, (8, 128), 0)
    lane = lax.broadcasted_iota(jnp.int32, (8, 128), 1)
    logits = {}
    routed = {}

    def router_tile(t, anchor=None):
        wr = jnp.broadcast_to(wr_ref[...].astype(_F32).reshape(1, D), (8, D))
        r = lax.dot_general(wr, xn[pl.ds(t * 128, 128), :].astype(_BF16), _NT,
                            preferred_element_type=_F32)
        b, row = divmod(t, 8)
        logits[b] = r if row == 0 else jnp.where(sub == row, r, logits[b])

    def top_c(anchor=None):
        vals, idxs = [], []
        for b in sorted(logits):
            v = _rnd(logits[b])
            vals.append(jnp.where(v != v, -jnp.inf, v))
            idxs.append((b * 1024 + sub * 128 + lane).astype(_F32))
        sel = []
        r_sel = jnp.zeros((_TOP_C, 128), _F32)
        for k in range(_TOP_C):
            m = functools.reduce(jnp.maximum, vals)
            m = jnp.max(jnp.max(m, axis=1, keepdims=True), axis=0, keepdims=True)
            cand = [jnp.where(v == m, i, float(S)) for v, i in zip(vals, idxs)]
            first = functools.reduce(jnp.minimum, cand)
            first = jnp.min(jnp.min(first, axis=1, keepdims=True), axis=0, keepdims=True)
            vals = [jnp.where(i == first, -jnp.inf, v) for v, i in zip(vals, idxs)]
            idxs = [jnp.where(i == first, float(S), i) for i in idxs]
            r_sel = jnp.where(sub == k, m, r_sel)
            sel.append(jnp.clip(first[0, 0].astype(jnp.int32), 0, S - 1))
        routed["sel"] = sel
        routed["r"] = r_sel[:, 0:1]
        routed["x"] = jnp.concatenate([xn[pl.ds(tok, 1), :] for tok in sel], axis=0)

    n_ffn = wg.shape[0]
    ffn_blocks = [(f0, min(_FFN_BLK, n_ffn - f0)) for f0 in range(0, n_ffn, _FFN_BLK)]

    def expert_hidden(n, anchor=None):
        f0, fn = ffn_blocks[n]
        hg = lax.dot_general(routed["x"], wg[pl.ds(f0, fn), :], _NT, preferred_element_type=_F32)
        hu = lax.dot_general(routed["x"], wu[pl.ds(f0, fn), :], _NT, preferred_element_type=_F32)
        routed[n] = _rnd(_silu(_rnd(hg))) * _rnd(hu)

    def expert_down(n, anchor=None):
        f0, fn = ffn_blocks[n]
        t = jnp.dot(routed.pop(n), wd[pl.ds(f0, fn), :], preferred_element_type=_F32)
        routed["y"] = t if n == 0 else routed["y"] + t

    def expert_scatter(anchor=None):
        y = _rnd(_rnd(routed["y"]) * _rnd(jax.nn.sigmoid(routed["r"])))
        rows = _rnd(routed["x"] + y)
        for k, tok in enumerate(routed["sel"]):
            xg[pl.ds(tok, 1), :] = rows[k:k + 1, :]

    per_grp = pre // _BULK_ROWS
    per_chunk = per_grp * (_CH // _G)
    n_slot = per_chunk * n_chunk
    waits = {per_chunk - per_grp: [w_cp[1], x_cp[1]] + small_cp,
             2 * per_chunk - per_grp: [w_cp[2], x_cp[2]],
             3 * per_chunk - per_grp: [w_cp[3], w_cp[4]],
             4 * per_chunk: ffn_cp,
             5 * per_chunk - per_grp: [w_cp[5]]}
    side = [[] for _ in range(n_slot)]

    def spread(tasks, first, last):
        for n, task in enumerate(tasks):
            side[first + n * (last - first + 1) // len(tasks)].append(task)

    def ln_tasks(part):
        r0, n = x_parts[part]
        return [functools.partial(layernorm, r) for r in range(r0, r0 + n, _LN_BLK)]

    def router_tasks(part):
        r0, n = x_parts[part]
        return [functools.partial(router_tile, t) for t in range(r0 // 128, (r0 + n) // 128)]

    for grp in range(1, n_slot // per_grp):
        for j in range(_G // 2):
            side[(grp - 1) * per_grp + j].append(functools.partial(
                retile, grp * (_G // 2) + j, d_lo=_D_SPLIT if grp < _CH // _G else 0))
    b1, b2, b3, b4, _ = sorted(waits)
    late_ln = ln_tasks(2)
    spread(ln_tasks(1), b1 + 1, b2 - 3)
    spread(router_tasks(0), b1 + 1, b2 - 3)
    spread(late_ln[:len(late_ln) // 2], b2 + 1, b3 - 3)
    spread(router_tasks(1), b2 + 1, b3 - 3)
    spread(late_ln[len(late_ln) // 2:], b3 + 1, b3 + 10)
    spread(router_tasks(2), b3 + 4, b4 - 7)
    side[b4 - 7].append(top_c)
    spread([functools.partial(fn, n) for n in range(len(ffn_blocks))
            for fn in (expert_hidden, expert_down)] + [expert_scatter], b4, n_slot - 3)

    x_cp[0].wait()
    for task in ln_tasks(0):
        task()
    w_first.wait()
    for pair in range(_CH // 2):
        retile(pair, d_hi=_D_SPLIT)
    for slot in range(per_chunk):
        j = slot - (per_chunk - per_grp)
        if j == 0:
            w_cp[0].wait()
        anchor = bulk(slot // per_grp, (slot % per_grp) * _BULK_ROWS, d_hi=_D_SPLIT)
        if 0 <= j < _G // 2:
            retile(j, anchor, d_lo=_D_SPLIT)
    for slot in range(n_slot):
        for cp in waits.get(slot, []):
            cp.wait()
        anchor = bulk(slot // per_grp, (slot % per_grp) * _BULK_ROWS,
                      d_lo=_D_SPLIT if slot < per_chunk else 0)
        for task in side[slot]:
            task(anchor)

    for cp in wo_cp:
        cp.wait()

    qi = lax.broadcasted_iota(jnp.int32, (L, L), 0)
    ki = lax.broadcasted_iota(jnp.int32, (L, L), 1)
    mask = (qi >= seg) | (ki >= seg) | (qi >= ki)
    scale = dh ** -0.5

    def finish(s):
        rows = pl.ds(pl.multiple_of(s * seg, seg), seg)
        sg = _rnd(_rnd(sbuf[...]) * _rnd(_silu(xg[rows, :])))
        obuf[rows, :] = (xb[rows, :].astype(_F32) + sg).astype(_BF16)

    def send(r0, n):
        pltpu.make_async_copy(obuf.at[pl.ds(r0, n)], out_hbm.at[pl.ds(r0, n)], osem).start()

    def step(s, mem):
        finish(jnp.maximum(s - 1, 0))
        xr = xn[pl.ds(pl.multiple_of(pre + s * xrows, 8), xrows), :]
        h = jnp.concatenate([xr, mem], axis=0).astype(_BF16)
        wpos = pl.ds(pl.multiple_of(lax.rem(s * xrows, ring_rows), 8), xrows)
        rpos = pl.ds(pl.multiple_of(lax.rem(s * seg + ring_off, ring_rows), 8), seg)
        xresult, presult, probs, heads_out = {}, {}, {}, {}
        acc = [None]

        def stage_a(g):
            ids = [m * heads + g * _G + j for m in range(3) for j in range(_G)]
            t = jnp.dot(h, weights(ids), preferred_element_type=_F32)
            for n, i in enumerate(ids):
                xresult[i] = t[:xrows, n * dh:(n + 1) * dh]
                presult[i] = t[xrows:, n * dh:(n + 1) * dh]

        def stage_w(g):
            for m in range(3):
                for j in range(_G):
                    i = m * heads + g * _G + j
                    ring[i, wpos, :] = xresult.pop(i)

        def rows_of(i):
            return jnp.concatenate([ring[i, rpos, :], presult[i]], axis=0)

        def stage_s(g):
            for j in range(_G):
                hd = g * _G + j
                k = rows_of(heads + hd).astype(_BF16)
                sc = lax.dot_general(rows_of(hd), k, _NT, preferred_element_type=_F32) * scale
                sc = jnp.where(mask, sc, -1000000000.0)
                e = jnp.exp(sc - jnp.max(sc, axis=-1, keepdims=True))
                probs[hd] = e * (1.0 / jnp.sum(e, axis=-1, keepdims=True))

        def stage_p(g):
            outs = []
            for j in range(_G):
                hd = g * _G + j
                v = rows_of(2 * heads + hd).astype(_BF16)
                outs.append(jnp.dot(probs.pop(hd), v, preferred_element_type=_F32))
            heads_out[g] = jnp.concatenate(outs, axis=1)

        def stage_o(g):
            n = _G * dh // 2
            wt = jnp.concatenate([wo[j, g * n:(g + 1) * n, :] for j in range(n_col)], axis=1)
            t = jnp.dot(heads_out[g], pltpu.bitcast(wt, _BF16), preferred_element_type=_F32)
            acc[0] = t if acc[0] is None else acc[0] + t

        stages = {"A": stage_a, "W": stage_w, "S": stage_s, "P": stage_p, "O": stage_o}
        for name, g in _schedule(ng):
            stages[name](g)
        sbuf[...] = acc[0][:seg]
        return acc[0][seg:]

    n_iter = n_seg // _UNROLL
    n_early = S - (_UNROLL + 1) * seg

    def steps(it, mem):
        for u in range(_UNROLL):
            mem = step(it * _UNROLL + u, mem)

        @pl.when(it == n_iter - 2)
        def _():
            send(0, n_early)

        return mem

    sbuf[...] = jnp.zeros(sbuf.shape, _F32)
    lax.fori_loop(0, n_iter, steps, mem0_ref[...].astype(_F32))
    send(n_early, S - n_early - seg)
    finish(n_seg - 1)
    send(S - seg, seg)
    pltpu.make_async_copy(obuf, obuf, osem).wait()


@functools.partial(jax.jit, static_argnames=("A_seg_len",))
def pallas_recurrent_scan__memory_aug_recurrent_mem_tr__moe_arch_mod__prompt_kernel(
    A_x, A_mem0, A_Wq, A_Wk, A_Wv, A_Wo, A_seg_len,
    B_x, B_w_r, B_w_gate, B_w_up, B_w_down,
):
    del B_x
    B, S, D = A_x.shape
    _, H, Dh = A_Wq.shape
    M = A_mem0.shape[1]
    F = B_w_gate.shape[1]
    seg = int(A_seg_len)
    assert B == 1 and S % seg == 0 and Dh == 128 and D % 128 == 0 and H % _CH == 0
    xrows = seg - M
    pre = S - (S // seg) * xrows
    lcm = int(np.lcm(seg, xrows))
    ring_rows = -(-(pre + xrows) // lcm) * lcm
    n_chunk = 3 * H // _CH
    n_sem = 3 + (n_chunk + 1) + D // 128 + 5

    hbm = pl.BlockSpec(memory_space=pltpu.HBM)
    out = pl.pallas_call(
        functools.partial(_kernel, seg=seg, n_mem=M, heads=H, dh=Dh),
        out_shape=jax.ShapeDtypeStruct((S, D), A_x.dtype),
        in_specs=[hbm] * 10,
        out_specs=hbm,
        scratch_shapes=[
            pltpu.VMEM((n_chunk, D * _CH // 2, Dh), _U32),
            pltpu.VMEM((F, D), _BF16),
            pltpu.VMEM((F, D), _BF16),
            pltpu.VMEM((F, D), _BF16),
            pltpu.VMEM((D,), _BF16),
            pltpu.VMEM((M, D), _BF16),
            pltpu.VMEM((pre // 2, D), _U32),
            pltpu.VMEM((3 * H, D // 2, Dh), _U32),
            pltpu.VMEM((D // 128, H * Dh // 2, 128), _U32),
            pltpu.VMEM((3 * H, ring_rows, Dh), _F32),
            pltpu.VMEM((S, D), _BF16),
            pltpu.VMEM((S, D), _BF16),
            pltpu.VMEM((S, D), _F32),
            pltpu.VMEM((S, D), _F32),
            pltpu.VMEM((seg, D), _F32),
            pltpu.SemaphoreType.DMA((n_sem,)),
            pltpu.SemaphoreType.DMA(()),
        ],
        compiler_params=pltpu.CompilerParams(vmem_limit_bytes=112 * 1024 * 1024),
    )(
        A_x.reshape(S, D), A_mem0.reshape(M, D), A_Wq, A_Wk, A_Wv, A_Wo.reshape(H * Dh, D),
        B_w_r, B_w_gate.T, B_w_up.T, B_w_down,
    )
    return out.reshape(B, S, D)
```

```python
import functools

import jax
import jax.numpy as jnp
import numpy as np
from jax import lax
from jax.experimental import pallas as pl
from jax.experimental.pallas import tpu as pltpu

_F32 = jnp.float32
_BF16 = jnp.bfloat16
_U32 = jnp.uint32
_NT = (((1,), (1,)), ((), ()))

_TOP_C = 8
_LN_EPS = 1e-05
_G = 4
_CH = 16
_LN_BLK = 32
_BULK_ROWS = 128
_UNROLL = 4
_D_SPLIT = 256
_FFN_BLK = 128


def _rnd(v):
    return v.astype(_BF16).astype(_F32)


def _silu(v):
    half = 0.5 * v
    return half * jnp.tanh(half) + half


def _after(v, anchor):
    if anchor is None:
        return v
    keep = (pltpu.bitcast(anchor, jnp.int32) | 1) != 0
    keep = jnp.tile(keep, (v.shape[0] // 8, v.shape[1] // 128))
    return jnp.where(keep, v, jnp.zeros_like(v))


def _schedule(ng):
    toks = []
    for g in range(ng):
        toks.append(("A", g))
        if g >= 1:
            toks.append(("S", g - 1))
        if g >= 2:
            toks.append(("P", g - 2))
        toks.append(("W", g))
    first, second = ng // 4, ng - 3 * ng // 8
    toks += [("O", g) for g in range(first)] + [("S", ng - 1), ("P", ng - 2)]
    toks += [("O", g) for g in range(first, second)] + [("P", ng - 1)]
    toks += [("O", g) for g in range(second, ng)]
    return toks


def _kernel(x_hbm, mem0_hbm, wq_hbm, wk_hbm, wv_hbm, wo_hbm, wr_hbm, wg_hbm, wu_hbm, wd_hbm,
            out_hbm,
            stg, wg, wu, wd, wr_ref, mem0_ref, xpre, w, wo, ring, xb, obuf, xg, xn, sbuf, sems, osem,
            *, seg, n_mem, heads, dh):
    S, D = xb.shape
    n_seg = S // seg
    L = seg + n_mem
    xrows = seg - n_mem
    pre = S - n_seg * xrows
    ring_rows = ring.shape[1]
    ring_off = ring_rows - pre
    n_chunk = 3 * heads // _CH
    n_col = D // 128
    ln_rows = (S - pre) // 4
    ng = heads // _G

    x_parts = [(0, pre), (pre, ln_rows), (pre + ln_rows, S - pre - ln_rows)]
    srcs = [(x_hbm.at[pl.ds(r0, n)], xb.at[pl.ds(r0, n)]) for r0, n in x_parts]
    for c, d0, d1 in [(0, 0, _D_SPLIT), (0, _D_SPLIT, D)] + [(c, 0, D) for c in range(1, n_chunk)]:
        src = (wq_hbm, wk_hbm, wv_hbm)[c // (heads // _CH)].bitcast(_U32)
        h2 = (c % (heads // _CH)) * (_CH // 2)
        srcs.append((src.at[pl.ds(d0, d1 - d0), pl.ds(h2, _CH // 2), :],
                     stg.at[c].reshape(D, _CH // 2, dh).at[pl.ds(d0, d1 - d0)]))
    wo32 = wo_hbm.bitcast(_U32)
    for j in range(n_col):
        srcs.append((wo32.at[:, pl.ds(j * 128, 128)], wo.at[j]))
    srcs += [(wg_hbm, wg), (wu_hbm, wu), (wd_hbm, wd), (wr_hbm, wr_ref), (mem0_hbm, mem0_ref)]
    copies = [pltpu.make_async_copy(a, b, sems.at[i]) for i, (a, b) in enumerate(srcs)]
    x_cp, copies = copies[:len(x_parts)], copies[len(x_parts):]
    w_first, w_cp, copies = copies[0], copies[1:n_chunk + 1], copies[n_chunk + 1:]
    wo_cp, copies = copies[:n_col], copies[n_col:]
    ffn_cp, small_cp = copies[:3], copies[3:]

    for cp in ([x_cp[0], w_first, w_cp[0]] + small_cp
               + [w_cp[1], x_cp[1], w_cp[2], x_cp[2], w_cp[3], w_cp[4]]
               + ffn_cp + [w_cp[5]] + wo_cp):
        cp.start()

    normalized = set()

    def layernorm(r0, anchor=None):
        normalized.add(r0)
        rows = pl.ds(r0, _LN_BLK)
        v = xb[rows, :].astype(_F32)
        v = jnp.concatenate([_after(v[:, :128], anchor), v[:, 128:]], axis=1)
        mean = jnp.mean(v, axis=-1, keepdims=True)
        dev = v - mean
        var = jnp.mean(dev * dev, axis=-1, keepdims=True)
        den = _rnd(jnp.sqrt(_rnd(_rnd(var) + _LN_EPS)))
        y = (_rnd(v - _rnd(mean)) * (1.0 / den)).astype(_BF16)
        if r0 < pre:
            xpre[pl.ds(r0 // 2, _LN_BLK // 2), :] = pltpu.bitcast(y, _U32)
        xn[rows, :] = y.astype(_F32)
        xg[rows, :] = y.astype(_F32)

    def retile(pair, anchor=None, d_lo=0, d_hi=D):
        c, j = divmod(pair, _CH // 2)
        blk = 128
        for d0 in range(d_lo, d_hi, blk):
            u = stg[c, pl.ds(d0 * (_CH // 2) + j, blk, stride=_CH // 2), :]
            lo = pltpu.bitcast(u.astype(jnp.uint16), _U32)
            hi = pltpu.bitcast((u >> 16).astype(jnp.uint16), _U32)
            w[2 * pair, pl.ds(d0 // 2, blk // 2), :] = lo
            w[2 * pair + 1, pl.ds(d0 // 2, blk // 2), :] = hi

    def weights(ids, d_lo=0, d_hi=D):
        rows = pl.ds(d_lo // 2, (d_hi - d_lo) // 2)
        return pltpu.bitcast(jnp.concatenate([w[i, rows, :] for i in ids], axis=1), _BF16)

    def bulk(grp, r0, d_lo=0, d_hi=D):
        ids = [grp * _G + j for j in range(_G)]
        lhs = pltpu.bitcast(xpre[pl.ds(r0 // 2, _BULK_ROWS // 2), d_lo:d_hi], _BF16)
        t = jnp.dot(lhs, weights(ids, d_lo, d_hi), preferred_element_type=_F32)
        rows = pl.ds(ring_off + r0, _BULK_ROWS)
        for j, i in enumerate(ids):
            part = t[:, j * dh:(j + 1) * dh]
            ring[i, rows, :] = part if d_lo == 0 else ring[i, rows, :] + part
        return t[:8, :128]

    sub = lax.broadcasted_iota(jnp.int32, (8, 128), 0)
    lane = lax.broadcasted_iota(jnp.int32, (8, 128), 1)
    logits = {}
    routed = {}

    def router_tile(t, anchor=None):
        assert normalized.issuperset(range(t * 128, (t + 1) * 128, _LN_BLK))
        wr = jnp.broadcast_to(wr_ref[...].astype(_F32).reshape(1, D), (8, D))
        r = lax.dot_general(wr, xn[pl.ds(t * 128, 128), :].astype(_BF16), _NT,
                            preferred_element_type=_F32)
        b, row = divmod(t, 8)
        logits[b] = r if row == 0 else jnp.where(sub == row, r, logits[b])

    def top_c(anchor=None):
        assert len(normalized) * _LN_BLK == S and len(logits) * 1024 == S
        vals, idxs = [], []
        for b in sorted(logits):
            v = _rnd(logits[b])
            vals.append(jnp.where(v != v, -jnp.inf, v))
            idxs.append((b * 1024 + sub * 128 + lane).astype(_F32))
        sel = []
        r_sel = jnp.zeros((_TOP_C, 128), _F32)
        for k in range(_TOP_C):
            m = functools.reduce(jnp.maximum, vals)
            m = jnp.max(jnp.max(m, axis=1, keepdims=True), axis=0, keepdims=True)
            cand = [jnp.where(v == m, i, float(S)) for v, i in zip(vals, idxs)]
            first = functools.reduce(jnp.minimum, cand)
            first = jnp.min(jnp.min(first, axis=1, keepdims=True), axis=0, keepdims=True)
            vals = [jnp.where(i == first, -jnp.inf, v) for v, i in zip(vals, idxs)]
            idxs = [jnp.where(i == first, float(S), i) for i in idxs]
            r_sel = jnp.where(sub == k, m, r_sel)
            sel.append(jnp.clip(first[0, 0].astype(jnp.int32), 0, S - 1))
        routed["sel"] = sel
        routed["r"] = r_sel[:, 0:1]
        routed["x"] = jnp.concatenate([xn[pl.ds(tok, 1), :] for tok in sel], axis=0)

    n_ffn = wg.shape[0]
    ffn_blocks = [(f0, min(_FFN_BLK, n_ffn - f0)) for f0 in range(0, n_ffn, _FFN_BLK)]

    def expert_hidden(n, anchor=None):
        f0, fn = ffn_blocks[n]
        hg = lax.dot_general(routed["x"], wg[pl.ds(f0, fn), :], _NT, preferred_element_type=_F32)
        hu = lax.dot_general(routed["x"], wu[pl.ds(f0, fn), :], _NT, preferred_element_type=_F32)
        routed[n] = _rnd(_silu(_rnd(hg))) * _rnd(hu)

    def expert_down(n, anchor=None):
        f0, fn = ffn_blocks[n]
        t = jnp.dot(routed.pop(n), wd[pl.ds(f0, fn), :], preferred_element_type=_F32)
        routed["y"] = t if n == 0 else routed["y"] + t

    def expert_scatter(anchor=None):
        y = _rnd(_rnd(routed["y"]) * _rnd(jax.nn.sigmoid(routed["r"])))
        rows = _rnd(routed["x"] + y)
        for k, tok in enumerate(routed["sel"]):
            xg[pl.ds(tok, 1), :] = rows[k:k + 1, :]

    per_grp = pre // _BULK_ROWS
    per_chunk = per_grp * (_CH // _G)
    n_slot = per_chunk * n_chunk
    waits = {per_chunk - per_grp: [w_cp[1], x_cp[1]] + small_cp,
             2 * per_chunk - per_grp: [w_cp[2], x_cp[2]],
             3 * per_chunk - per_grp: [w_cp[3], w_cp[4]],
             4 * per_chunk: ffn_cp,
             5 * per_chunk - per_grp: [w_cp[5]]}
    side = [[] for _ in range(n_slot)]

    def spread(tasks, first, last):
        for n, task in enumerate(tasks):
            side[first + n * (last - first + 1) // len(tasks)].append(task)

    def ln_tasks(part):
        r0, n = x_parts[part]
        return [functools.partial(layernorm, r) for r in range(r0, r0 + n, _LN_BLK)]

    def router_tasks(part):
        r0, n = x_parts[part]
        return [functools.partial(router_tile, t) for t in range(r0 // 128, (r0 + n) // 128)]

    for grp in range(1, n_slot // per_grp):
        for j in range(_G // 2):
            side[(grp - 1) * per_grp + j].append(functools.partial(
                retile, grp * (_G // 2) + j, d_lo=_D_SPLIT if grp < _CH // _G else 0))
    b1, b2, b3, b4, _ = sorted(waits)
    late_ln = ln_tasks(2)
    spread(ln_tasks(1), b1 + 1, b2 - 3)
    spread(router_tasks(0), b1 + 1, b2 - 3)
    spread(late_ln[:len(late_ln) // 2], b2 + 1, b3 - 3)
    spread(router_tasks(1), b2 + 1, b3 - 3)
    spread(late_ln[len(late_ln) // 2:], b3 + 1, b3 + 10)
    spread(router_tasks(2), b3 + 4, b4 - 7)
    side[b4 - 7].append(top_c)
    spread([functools.partial(fn, n) for n in range(len(ffn_blocks))
            for fn in (expert_hidden, expert_down)] + [expert_scatter], b4, n_slot - 3)

    x_cp[0].wait()
    for task in ln_tasks(0):
        task()
    w_first.wait()
    for pair in range(_CH // 2):
        retile(pair, d_hi=_D_SPLIT)
    for slot in range(per_chunk):
        j = slot - (per_chunk - per_grp)
        if j == 0:
            w_cp[0].wait()
        anchor = bulk(slot // per_grp, (slot % per_grp) * _BULK_ROWS, d_hi=_D_SPLIT)
        if 0 <= j < _G // 2:
            retile(j, anchor, d_lo=_D_SPLIT)
    for slot in range(n_slot):
        for cp in waits.get(slot, []):
            cp.wait()
        anchor = bulk(slot // per_grp, (slot % per_grp) * _BULK_ROWS,
                      d_lo=_D_SPLIT if slot < per_chunk else 0)
        for task in side[slot]:
            task(anchor)

    for cp in wo_cp:
        cp.wait()

    qi = lax.broadcasted_iota(jnp.int32, (L, L), 0)
    ki = lax.broadcasted_iota(jnp.int32, (L, L), 1)
    mask = (qi >= seg) | (ki >= seg) | (qi >= ki)
    scale = dh ** -0.5

    def finish(s):
        rows = pl.ds(pl.multiple_of(s * seg, seg), seg)
        sg = _rnd(_rnd(sbuf[...]) * _rnd(_silu(xg[rows, :])))
        obuf[rows, :] = (xb[rows, :].astype(_F32) + sg).astype(_BF16)

    def send(r0, n):
        pltpu.make_async_copy(obuf.at[pl.ds(r0, n)], out_hbm.at[pl.ds(r0, n)], osem).start()

    def step(s, mem):
        finish(jnp.maximum(s - 1, 0))
        xr = xn[pl.ds(pl.multiple_of(pre + s * xrows, 8), xrows), :]
        h = jnp.concatenate([xr, mem], axis=0).astype(_BF16)
        wpos = pl.ds(pl.multiple_of(lax.rem(s * xrows, ring_rows), 8), xrows)
        rpos = pl.ds(pl.multiple_of(lax.rem(s * seg + ring_off, ring_rows), 8), seg)
        xresult, presult, probs, heads_out = {}, {}, {}, {}
        acc = [None]

        def stage_a(g):
            ids = [m * heads + g * _G + j for m in range(3) for j in range(_G)]
            t = jnp.dot(h, weights(ids), preferred_element_type=_F32)
            for n, i in enumerate(ids):
                xresult[i] = t[:xrows, n * dh:(n + 1) * dh]
                presult[i] = t[xrows:, n * dh:(n + 1) * dh]

        def stage_w(g):
            for m in range(3):
                for j in range(_G):
                    i = m * heads + g * _G + j
                    ring[i, wpos, :] = xresult.pop(i)

        def rows_of(i):
            return jnp.concatenate([ring[i, rpos, :], presult[i]], axis=0)

        def stage_s(g):
            for j in range(_G):
                hd = g * _G + j
                k = rows_of(heads + hd).astype(_BF16)
                sc = lax.dot_general(rows_of(hd), k, _NT, preferred_element_type=_F32) * scale
                sc = jnp.where(mask, sc, -1000000000.0)
                e = jnp.exp(sc - jnp.max(sc, axis=-1, keepdims=True))
                probs[hd] = e * (1.0 / jnp.sum(e, axis=-1, keepdims=True))

        def stage_p(g):
            outs = []
            for j in range(_G):
                hd = g * _G + j
                v = rows_of(2 * heads + hd).astype(_BF16)
                outs.append(jnp.dot(probs.pop(hd), v, preferred_element_type=_F32))
            heads_out[g] = jnp.concatenate(outs, axis=1)

        def stage_o(g):
            n = _G * dh // 2
            wt = jnp.concatenate([wo[j, g * n:(g + 1) * n, :] for j in range(n_col)], axis=1)
            t = jnp.dot(heads_out[g], pltpu.bitcast(wt, _BF16), preferred_element_type=_F32)
            acc[0] = t if acc[0] is None else acc[0] + t

        stages = {"A": stage_a, "W": stage_w, "S": stage_s, "P": stage_p, "O": stage_o}
        for name, g in _schedule(ng):
            stages[name](g)
        sbuf[...] = acc[0][:seg]
        return acc[0][seg:]

    n_iter = n_seg // _UNROLL
    n_early = S - (_UNROLL + 1) * seg

    def steps(it, mem):
        for u in range(_UNROLL):
            mem = step(it * _UNROLL + u, mem)

        @pl.when(it == n_iter - 2)
        def _():
            send(0, n_early)

        return mem

    sbuf[...] = jnp.zeros(sbuf.shape, _F32)
    lax.fori_loop(0, n_iter, steps, mem0_ref[...].astype(_F32))
    send(n_early, S - n_early - seg)
    finish(n_seg - 1)
    send(S - seg, seg)
    pltpu.make_async_copy(obuf, obuf, osem).wait()


@functools.partial(jax.jit, static_argnames=("A_seg_len",))
def pallas_recurrent_scan__memory_aug_recurrent_mem_tr__moe_arch_mod__prompt_kernel(
    A_x, A_mem0, A_Wq, A_Wk, A_Wv, A_Wo, A_seg_len,
    B_x, B_w_r, B_w_gate, B_w_up, B_w_down,
):
    del B_x
    B, S, D = A_x.shape
    _, H, Dh = A_Wq.shape
    M = A_mem0.shape[1]
    F = B_w_gate.shape[1]
    seg = int(A_seg_len)
    assert B == 1 and Dh == 128 and D % 128 == 0 and H == 2 * _CH
    assert S % (seg * _UNROLL) == 0 and S % 1024 == 0 and M % 8 == 0 and seg % 16 == 0
    xrows = seg - M
    pre = S - (S // seg) * xrows
    lcm = int(np.lcm(seg, xrows))
    ring_rows = -(-(pre + xrows) // lcm) * lcm
    n_chunk = 3 * H // _CH
    n_sem = 3 + (n_chunk + 1) + D // 128 + 5

    hbm = pl.BlockSpec(memory_space=pltpu.HBM)
    out = pl.pallas_call(
        functools.partial(_kernel, seg=seg, n_mem=M, heads=H, dh=Dh),
        out_shape=jax.ShapeDtypeStruct((S, D), A_x.dtype),
        in_specs=[hbm] * 10,
        out_specs=hbm,
        scratch_shapes=[
            pltpu.VMEM((n_chunk, D * _CH // 2, Dh), _U32),
            pltpu.VMEM((F, D), _BF16),
            pltpu.VMEM((F, D), _BF16),
            pltpu.VMEM((F, D), _BF16),
            pltpu.VMEM((D,), _BF16),
            pltpu.VMEM((M, D), _BF16),
            pltpu.VMEM((pre // 2, D), _U32),
            pltpu.VMEM((3 * H, D // 2, Dh), _U32),
            pltpu.VMEM((D // 128, H * Dh // 2, 128), _U32),
            pltpu.VMEM((3 * H, ring_rows, Dh), _F32),
            pltpu.VMEM((S, D), _BF16),
            pltpu.VMEM((S, D), _BF16),
            pltpu.VMEM((S, D), _F32),
            pltpu.VMEM((S, D), _F32),
            pltpu.VMEM((seg, D), _F32),
            pltpu.SemaphoreType.DMA((n_sem,)),
            pltpu.SemaphoreType.DMA(()),
        ],
        compiler_params=pltpu.CompilerParams(vmem_limit_bytes=112 * 1024 * 1024),
    )(
        A_x.reshape(S, D), A_mem0.reshape(M, D), A_Wq, A_Wk, A_Wv, A_Wo.reshape(H * Dh, D),
        B_w_r, B_w_gate.T, B_w_up.T, B_w_down,
    )
    return out.reshape(B, S, D)
```

```python
import functools

import jax
import jax.numpy as jnp
import numpy as np
from jax import lax
from jax.experimental import pallas as pl
from jax.experimental.pallas import tpu as pltpu

_F32 = jnp.float32
_BF16 = jnp.bfloat16
_U32 = jnp.uint32
_NT = (((1,), (1,)), ((), ()))

_TOP_C = 8
_LN_EPS = 1e-05
_G = 4
_CH = 16
_LN_BLK = 32
_BULK_ROWS = 128
_UNROLL = 4
_D_SPLIT = 256
_FFN_BLK = 128


def _rnd(v):
    return v.astype(_BF16).astype(_F32)


def _silu(v):
    half = 0.5 * v
    return half * jnp.tanh(half) + half


def _after(v, anchor):
    if anchor is None:
        return v
    keep = (pltpu.bitcast(anchor, jnp.int32) | 1) != 0
    keep = jnp.tile(keep, (v.shape[0] // 8, v.shape[1] // 128))
    return jnp.where(keep, v, jnp.zeros_like(v))


def _schedule(ng):
    toks = []
    for g in range(ng):
        toks.append(("A", g))
        if g >= 1:
            toks.append(("S", g - 1))
        if g >= 2:
            toks.append(("P", g - 2))
        toks.append(("W", g))
    first, second = ng // 4, ng - 3 * ng // 8
    toks += [("O", g) for g in range(first)] + [("S", ng - 1), ("P", ng - 2)]
    toks += [("O", g) for g in range(first, second)] + [("P", ng - 1)]
    toks += [("O", g) for g in range(second, ng)]
    return toks


def _kernel(x_hbm, mem0_hbm, wq_hbm, wk_hbm, wv_hbm, wo_hbm, wr_hbm, wg_hbm, wu_hbm, wd_hbm,
            out_hbm,
            stg, wg, wu, wd, wr_ref, mem0_ref, xpre, w, wo, ring, xb, obuf, xg, xn, sbuf, sems, osem,
            *, seg, n_mem, heads, dh):
    S, D = xb.shape
    n_seg = S // seg
    L = seg + n_mem
    xrows = seg - n_mem
    pre = S - n_seg * xrows
    ring_rows = ring.shape[1]
    ring_off = ring_rows - pre
    n_chunk = 3 * heads // _CH
    n_col = D // 128
    ln_rows = (S - pre) // 4
    ng = heads // _G

    x_parts = [(0, pre), (pre, ln_rows), (pre + ln_rows, S - pre - ln_rows)]
    srcs = [(x_hbm.at[pl.ds(r0, n)], xb.at[pl.ds(r0, n)]) for r0, n in x_parts]
    for c, d0, d1 in [(0, 0, _D_SPLIT), (0, _D_SPLIT, D)] + [(c, 0, D) for c in range(1, n_chunk)]:
        src = (wq_hbm, wk_hbm, wv_hbm)[c // (heads // _CH)].bitcast(_U32)
        h2 = (c % (heads // _CH)) * (_CH // 2)
        srcs.append((src.at[pl.ds(d0, d1 - d0), pl.ds(h2, _CH // 2), :],
                     stg.at[c].reshape(D, _CH // 2, dh).at[pl.ds(d0, d1 - d0)]))
    wo32 = wo_hbm.bitcast(_U32)
    for j in range(n_col):
        srcs.append((wo32.at[:, pl.ds(j * 128, 128)], wo.at[j]))
    srcs += [(wg_hbm, wg), (wu_hbm, wu), (wd_hbm, wd), (wr_hbm, wr_ref), (mem0_hbm, mem0_ref)]
    copies = [pltpu.make_async_copy(a, b, sems.at[i]) for i, (a, b) in enumerate(srcs)]
    x_cp, copies = copies[:len(x_parts)], copies[len(x_parts):]
    w_first, w_cp, copies = copies[0], copies[1:n_chunk + 1], copies[n_chunk + 1:]
    wo_cp, copies = copies[:n_col], copies[n_col:]
    ffn_cp, small_cp = copies[:3], copies[3:]

    for cp in ([x_cp[0], w_first, w_cp[0]] + small_cp
               + [w_cp[1], x_cp[1], w_cp[2], x_cp[2], w_cp[3], w_cp[4]]
               + ffn_cp + [w_cp[5]] + wo_cp):
        cp.start()

    normalized = set()

    def layernorm(r0, anchor=None):
        normalized.add(r0)
        rows = pl.ds(r0, _LN_BLK)
        v = xb[rows, :].astype(_F32)
        v = jnp.concatenate([_after(v[:, :128], anchor), v[:, 128:]], axis=1)
        mean = jnp.mean(v, axis=-1, keepdims=True)
        dev = v - mean
        var = jnp.mean(dev * dev, axis=-1, keepdims=True)
        den = _rnd(jnp.sqrt(_rnd(_rnd(var) + _LN_EPS)))
        y = (_rnd(v - _rnd(mean)) * (1.0 / den)).astype(_BF16)
        if r0 < pre:
            xpre[pl.ds(r0 // 2, _LN_BLK // 2), :] = pltpu.bitcast(y, _U32)
        xn[rows, :] = y.astype(_F32)
        xg[rows, :] = y.astype(_F32)

    def retile(pair, anchor=None, d_lo=0, d_hi=D):
        c, j = divmod(pair, _CH // 2)
        blk = 128
        for d0 in range(d_lo, d_hi, blk):
            u = stg[c, pl.ds(d0 * (_CH // 2) + j, blk, stride=_CH // 2), :]
            lo = pltpu.bitcast(u.astype(jnp.uint16), _U32)
            hi = pltpu.bitcast((u >> 16).astype(jnp.uint16), _U32)
            w[2 * pair, pl.ds(d0 // 2, blk // 2), :] = lo
            w[2 * pair + 1, pl.ds(d0 // 2, blk // 2), :] = hi

    def weights(ids, d_lo=0, d_hi=D):
        rows = pl.ds(d_lo // 2, (d_hi - d_lo) // 2)
        return pltpu.bitcast(jnp.concatenate([w[i, rows, :] for i in ids], axis=1), _BF16)

    def bulk(grp, r0, d_lo=0, d_hi=D):
        ids = [grp * _G + j for j in range(_G)]
        lhs = pltpu.bitcast(xpre[pl.ds(r0 // 2, _BULK_ROWS // 2), d_lo:d_hi], _BF16)
        t = jnp.dot(lhs, weights(ids, d_lo, d_hi), preferred_element_type=_F32)
        rows = pl.ds(ring_off + r0, _BULK_ROWS)
        for j, i in enumerate(ids):
            part = t[:, j * dh:(j + 1) * dh]
            ring[i, rows, :] = part if d_lo == 0 else ring[i, rows, :] + part
        return t[:8, :128]

    sub = lax.broadcasted_iota(jnp.int32, (8, 128), 0)
    lane = lax.broadcasted_iota(jnp.int32, (8, 128), 1)
    logits = {}
    routed = {}

    def router_tile(t, anchor=None):
        assert normalized.issuperset(range(t * 128, (t + 1) * 128, _LN_BLK))
        wr = jnp.broadcast_to(wr_ref[...].astype(_F32).reshape(1, D), (8, D))
        r = lax.dot_general(wr, xn[pl.ds(t * 128, 128), :].astype(_BF16), _NT,
                            preferred_element_type=_F32)
        b, row = divmod(t, 8)
        logits[b] = r if row == 0 else jnp.where(sub == row, r, logits[b])

    def top_c(anchor=None):
        assert len(normalized) * _LN_BLK == S and len(logits) * 1024 == S
        vals, idxs = [], []
        for b in sorted(logits):
            v = _rnd(logits[b])
            vals.append(jnp.where(v != v, -jnp.inf, v))
            idxs.append((b * 1024 + sub * 128 + lane).astype(_F32))
        sel = []
        r_sel = jnp.zeros((_TOP_C, 128), _F32)
        for k in range(_TOP_C):
            m = functools.reduce(jnp.maximum, vals)
            m = jnp.max(jnp.max(m, axis=1, keepdims=True), axis=0, keepdims=True)
            cand = [jnp.where(v == m, i, float(S)) for v, i in zip(vals, idxs)]
            first = functools.reduce(jnp.minimum, cand)
            first = jnp.min(jnp.min(first, axis=1, keepdims=True), axis=0, keepdims=True)
            vals = [jnp.where(i == first, -jnp.inf, v) for v, i in zip(vals, idxs)]
            idxs = [jnp.where(i == first, float(S), i) for i in idxs]
            r_sel = jnp.where(sub == k, m, r_sel)
            sel.append(jnp.clip(first[0, 0].astype(jnp.int32), 0, S - 1))
        routed["sel"] = sel
        routed["r"] = r_sel[:, 0:1]
        routed["x"] = jnp.concatenate([xn[pl.ds(tok, 1), :] for tok in sel], axis=0)

    n_ffn = wg.shape[0]
    ffn_blocks = [(f0, min(_FFN_BLK, n_ffn - f0)) for f0 in range(0, n_ffn, _FFN_BLK)]

    def expert_hidden(n, anchor=None):
        f0, fn = ffn_blocks[n]
        hg = lax.dot_general(routed["x"], wg[pl.ds(f0, fn), :], _NT, preferred_element_type=_F32)
        hu = lax.dot_general(routed["x"], wu[pl.ds(f0, fn), :], _NT, preferred_element_type=_F32)
        routed[n] = _rnd(_silu(_rnd(hg))) * _rnd(hu)

    def expert_down(n, anchor=None):
        f0, fn = ffn_blocks[n]
        t = jnp.dot(routed.pop(n), wd[pl.ds(f0, fn), :], preferred_element_type=_F32)
        routed["y"] = t if n == 0 else routed["y"] + t

    def expert_scatter(anchor=None):
        y = _rnd(_rnd(routed["y"]) * _rnd(jax.nn.sigmoid(routed["r"])))
        rows = _rnd(routed["x"] + y)
        for k, tok in enumerate(routed["sel"]):
            xg[pl.ds(tok, 1), :] = rows[k:k + 1, :]

    per_grp = pre // _BULK_ROWS
    per_chunk = per_grp * (_CH // _G)
    n_slot = per_chunk * n_chunk
    waits = {per_chunk - per_grp: [w_cp[1], x_cp[1]] + small_cp,
             2 * per_chunk - per_grp: [w_cp[2], x_cp[2]],
             3 * per_chunk - per_grp: [w_cp[3], w_cp[4]],
             4 * per_chunk: ffn_cp,
             5 * per_chunk - per_grp: [w_cp[5]]}
    side = [[] for _ in range(n_slot)]

    def spread(tasks, first, last):
        for n, task in enumerate(tasks):
            side[first + n * (last - first + 1) // len(tasks)].append(task)

    def ln_tasks(part):
        r0, n = x_parts[part]
        return [functools.partial(layernorm, r) for r in range(r0, r0 + n, _LN_BLK)]

    def router_tasks(part):
        r0, n = x_parts[part]
        return [functools.partial(router_tile, t) for t in range(r0 // 128, (r0 + n) // 128)]

    for grp in range(1, n_slot // per_grp):
        for j in range(_G // 2):
            side[(grp - 1) * per_grp + j].append(functools.partial(
                retile, grp * (_G // 2) + j, d_lo=_D_SPLIT if grp < _CH // _G else 0))
    b1, b2, b3, b4, _ = sorted(waits)
    late_ln = ln_tasks(2)
    spread(ln_tasks(1), b1 + 1, b2 - 3)
    spread(router_tasks(0), b1 + 1, b2 - 3)
    spread(late_ln[:len(late_ln) // 2], b2 + 1, b3 - 3)
    spread(router_tasks(1), b2 + 1, b3 - 3)
    spread(late_ln[len(late_ln) // 2:], b3 + 1, b3 + 10)
    spread(router_tasks(2), b3 + 4, b4 - 7)
    side[b4 - 7].append(top_c)
    spread([functools.partial(fn, n) for n in range(len(ffn_blocks))
            for fn in (expert_hidden, expert_down)] + [expert_scatter], b4, n_slot - 3)

    x_cp[0].wait()
    for task in ln_tasks(0):
        task()
    w_first.wait()
    for pair in range(_CH // 2):
        retile(pair, d_hi=_D_SPLIT)
    for slot in range(per_chunk):
        j = slot - (per_chunk - per_grp)
        if j == 0:
            w_cp[0].wait()
        anchor = bulk(slot // per_grp, (slot % per_grp) * _BULK_ROWS, d_hi=_D_SPLIT)
        if 0 <= j < _G // 2:
            retile(j, anchor, d_lo=_D_SPLIT)
    for slot in range(n_slot):
        for cp in waits.get(slot, []):
            cp.wait()
        anchor = bulk(slot // per_grp, (slot % per_grp) * _BULK_ROWS,
                      d_lo=_D_SPLIT if slot < per_chunk else 0)
        for task in side[slot]:
            task(anchor)

    for cp in wo_cp:
        cp.wait()

    qi = lax.broadcasted_iota(jnp.int32, (L, L), 0)
    ki = lax.broadcasted_iota(jnp.int32, (L, L), 1)
    mask = (qi < n_mem) | (ki >= seg) | (qi - n_mem >= ki)
    scale = dh ** -0.5

    def finish(s):
        rows = pl.ds(pl.multiple_of(s * seg, seg), seg)
        sg = _rnd(_rnd(sbuf[...]) * _rnd(_silu(xg[rows, :])))
        obuf[rows, :] = (xb[rows, :].astype(_F32) + sg).astype(_BF16)

    def send(r0, n):
        pltpu.make_async_copy(obuf.at[pl.ds(r0, n)], out_hbm.at[pl.ds(r0, n)], osem).start()

    def step(s, mem):
        finish(jnp.maximum(s - 1, 0))
        xr = xn[pl.ds(pl.multiple_of(pre + s * xrows, 8), xrows), :]
        h = jnp.concatenate([xr, mem], axis=0).astype(_BF16)
        wpos = pl.ds(pl.multiple_of(lax.rem(s * xrows, ring_rows), 8), xrows)
        rpos = pl.ds(pl.multiple_of(lax.rem(s * seg + ring_off, ring_rows), 8), seg)
        xresult, presult, probs, heads_out = {}, {}, {}, {}
        acc = [None]

        def stage_a(g):
            ids = [m * heads + g * _G + j for m in range(3) for j in range(_G)]
            t = jnp.dot(h, weights(ids), preferred_element_type=_F32)
            for n, i in enumerate(ids):
                xresult[i] = t[:xrows, n * dh:(n + 1) * dh]
                presult[i] = t[xrows:, n * dh:(n + 1) * dh]

        def stage_w(g):
            for m in range(3):
                for j in range(_G):
                    i = m * heads + g * _G + j
                    ring[i, wpos, :] = xresult.pop(i)

        def rows_of(i):
            return jnp.concatenate([ring[i, rpos, :], presult[i]], axis=0)

        def stage_s(g):
            for j in range(_G):
                hd = g * _G + j
                k = rows_of(heads + hd).astype(_BF16)
                q = jnp.concatenate([presult[hd], ring[hd, rpos, :]], axis=0)
                sc = lax.dot_general(q, k, _NT, preferred_element_type=_F32) * scale
                sc = jnp.where(mask, sc, -1000000000.0)
                e = jnp.exp(sc - jnp.max(sc, axis=-1, keepdims=True))
                probs[hd] = e / jnp.sum(e, axis=-1, keepdims=True)

        def stage_p(g):
            outs = []
            for j in range(_G):
                hd = g * _G + j
                v = rows_of(2 * heads + hd).astype(_BF16)
                outs.append(jnp.dot(probs.pop(hd), v, preferred_element_type=_F32))
            heads_out[g] = jnp.concatenate(outs, axis=1)

        def stage_o(g):
            n = _G * dh // 2
            wt = jnp.concatenate([wo[j, g * n:(g + 1) * n, :] for j in range(n_col)], axis=1)
            t = jnp.dot(heads_out[g], pltpu.bitcast(wt, _BF16), preferred_element_type=_F32)
            acc[0] = t if acc[0] is None else acc[0] + t

        stages = {"A": stage_a, "W": stage_w, "S": stage_s, "P": stage_p, "O": stage_o}
        for name, g in _schedule(ng):
            stages[name](g)
        sbuf[...] = acc[0][n_mem:]
        return acc[0][:n_mem]

    n_iter = n_seg // _UNROLL
    n_early = S - (_UNROLL + 1) * seg

    def steps(it, mem):
        for u in range(_UNROLL):
            mem = step(it * _UNROLL + u, mem)

        @pl.when(it == n_iter - 2)
        def _():
            send(0, n_early)

        return mem

    sbuf[...] = jnp.zeros(sbuf.shape, _F32)
    lax.fori_loop(0, n_iter, steps, mem0_ref[...].astype(_F32))
    send(n_early, S - n_early - seg)
    finish(n_seg - 1)
    send(S - seg, seg)
    pltpu.make_async_copy(obuf, obuf, osem).wait()


@functools.partial(jax.jit, static_argnames=("A_seg_len",))
def pallas_recurrent_scan__memory_aug_recurrent_mem_tr__moe_arch_mod__prompt_kernel(
    A_x, A_mem0, A_Wq, A_Wk, A_Wv, A_Wo, A_seg_len,
    B_x, B_w_r, B_w_gate, B_w_up, B_w_down,
):
    del B_x
    B, S, D = A_x.shape
    _, H, Dh = A_Wq.shape
    M = A_mem0.shape[1]
    F = B_w_gate.shape[1]
    seg = int(A_seg_len)
    assert B == 1 and Dh == 128 and D % 128 == 0 and H == 2 * _CH
    assert S % (seg * _UNROLL) == 0 and S % 1024 == 0 and M % 8 == 0 and seg % 16 == 0
    xrows = seg - M
    pre = S - (S // seg) * xrows
    lcm = int(np.lcm(seg, xrows))
    ring_rows = -(-(pre + xrows) // lcm) * lcm
    n_chunk = 3 * H // _CH
    n_sem = 3 + (n_chunk + 1) + D // 128 + 5

    hbm = pl.BlockSpec(memory_space=pltpu.HBM)
    out = pl.pallas_call(
        functools.partial(_kernel, seg=seg, n_mem=M, heads=H, dh=Dh),
        out_shape=jax.ShapeDtypeStruct((S, D), A_x.dtype),
        in_specs=[hbm] * 10,
        out_specs=hbm,
        scratch_shapes=[
            pltpu.VMEM((n_chunk, D * _CH // 2, Dh), _U32),
            pltpu.VMEM((F, D), _BF16),
            pltpu.VMEM((F, D), _BF16),
            pltpu.VMEM((F, D), _BF16),
            pltpu.VMEM((D,), _BF16),
            pltpu.VMEM((M, D), _BF16),
            pltpu.VMEM((pre // 2, D), _U32),
            pltpu.VMEM((3 * H, D // 2, Dh), _U32),
            pltpu.VMEM((D // 128, H * Dh // 2, 128), _U32),
            pltpu.VMEM((3 * H, ring_rows, Dh), _F32),
            pltpu.VMEM((S, D), _BF16),
            pltpu.VMEM((S, D), _BF16),
            pltpu.VMEM((S, D), _F32),
            pltpu.VMEM((S, D), _F32),
            pltpu.VMEM((seg, D), _F32),
            pltpu.SemaphoreType.DMA((n_sem,)),
            pltpu.SemaphoreType.DMA(()),
        ],
        compiler_params=pltpu.CompilerParams(vmem_limit_bytes=112 * 1024 * 1024),
    )(
        A_x.reshape(S, D), A_mem0.reshape(M, D), A_Wq, A_Wk, A_Wv, A_Wo.reshape(H * Dh, D),
        B_w_r, B_w_gate.T, B_w_up.T, B_w_down,
    )
    return out.reshape(B, S, D)
```
